```python
import os as _os
_os.environ.setdefault("JAX_PLATFORMS", "cpu")
import jax
import jax.numpy as jnp

def _softmax(x, axis=-1):
    return jax.nn.softmax(x, axis=axis)
def _gelu(x):
    return jax.nn.gelu(x, approximate=True)
def _silu(x):
    return jax.nn.silu(x)
def _sigmoid(x):
    return jax.nn.sigmoid(x)
def _layernorm(x, axis=-1, eps=1e-5):
    m = jnp.mean(x, axis=axis, keepdims=True)
    v = jnp.var(x, axis=axis, keepdims=True)
    return (x - m) / jnp.sqrt(v + eps)
def _scatter_add(tgt, idx, src, axis=0):
    return tgt.at[idx].add(src)
def _segment_sum(src, seg, n):
    return jax.ops.segment_sum(src, seg, n)
class _Rng:
    def __init__(self, key):
        self._k = key
    def _next(self):
        self._k, sub = jax.random.split(self._k)
        return sub
    def normal(self, shape):
        return jax.random.normal(self._next(), shape, dtype=jnp.bfloat16)
    def randint(self, lo, hi, shape):
        return jax.random.randint(self._next(), shape, lo, hi, dtype=jnp.int32)
    def uniform(self, shape, lo=0.0, hi=1.0):
        return jax.random.uniform(self._next(), shape, jnp.bfloat16, lo, hi)
    def permutation(self, n):
        return jax.random.permutation(self._next(), n)


kernel_name = 'interleave_layers__grouped_kv_mqa__sliding_block__prompt'

def setup_inputs():
    _rng = _Rng(jax.random.key(int.from_bytes(__import__("os").urandom(4), "little")))
    _w = (lambda a: (lambda t: t.astype(jnp.bfloat16) if jnp.issubdtype(t.dtype, jnp.floating) else t)(jnp.asarray(a)))
    def _A_setup():
        B, S, D, H = 1, 2048, 448, 16
        Dh = D // H
        return {
            "x": _w((lambda *s: _rng.normal(s) * 0.05)(B, S, D)),
            "wq": _w((lambda *s: _rng.normal(s) * 0.05)(D, H * Dh)),
            "wk": _w((lambda *s: _rng.normal(s) * 0.05)(D, Dh)),
            "wv": _w((lambda *s: _rng.normal(s) * 0.05)(D, Dh)),
            "wo": _w((lambda *s: _rng.normal(s) * 0.05)(H * Dh, D)),
        }
    _A_in = _A_setup()

    def _B_setup():
        B, S, D = 1, 2048, 448
        return {
            "x": _w((lambda *s: _rng.normal(s) * 0.05)(B, S, D)),
            "wqkv": _w((lambda *s: _rng.normal(s) * 0.05)(D, 3 * D)),
            "wo": _w((lambda *s: _rng.normal(s) * 0.05)(D, D)),
        }
    _B_in = _B_setup()

    return {
        "A_x": _A_in["x"],
        "A_wq": _A_in["wq"],
        "A_wk": _A_in["wk"],
        "A_wv": _A_in["wv"],
        "A_wo": _A_in["wo"],
        "B_x": _B_in["x"],
        "B_wqkv": _B_in["wqkv"],
        "B_wo": _B_in["wo"],
    }

def reference(A_x, A_wq, A_wk, A_wv, A_wo, B_x, B_wqkv, B_wo):
    def _A_ref(x, wq, wk, wv, wo):
        B, S, D = x.shape
        H = 16
        Dh = D // H
        q = (lambda x, *d: x.transpose(*d))((x @ wq).reshape(B, S, H, Dh), 0, 2, 1, 3)
        k = x @ wk
        v = x @ wv
        scores = jnp.einsum("bhqd,bkd->bhqk", q, k) * (Dh ** -0.5)
        p = _softmax(scores, axis=-1)
        o = jnp.einsum("bhqk,bkd->bhqd", p, v)
        return (lambda x, *d: x.transpose(*d))(o, 0, 2, 1, 3).reshape(B, S, H * Dh) @ wo

    def _B_ref(x, wqkv, wo):
        B, S, D = x.shape
        H = 16; Dh = D // H; W = 256
        qkv = (lambda x, *d: x.transpose(*d))((x @ wqkv).reshape(B, S, 3, H, Dh), 2, 0, 3, 1, 4)
        q, k, v = qkv[0], qkv[1], qkv[2]
        scores = jnp.einsum("bhqd,bhkd->bhqk", q, k) * (Dh ** -0.5)
        idx = jnp.arange(S)
        mask = (idx[:, None] - idx[None, :] >= 0) & (idx[:, None] - idx[None, :] < W)
        scores = jnp.where(mask[None, None], scores, -1e9)
        p = _softmax(scores, axis=-1)
        o = jnp.einsum("bhqk,bhkd->bhqd", p, v)
        return (lambda x, *d: x.transpose(*d))(o, 0, 2, 1, 3).reshape(B, S, D) @ wo

    x = A_x
    x = x + _A_ref(_layernorm(x, axis=-1), A_wq, A_wk, A_wv, A_wo)
    x = x + _B_ref(_layernorm(x, axis=-1), B_wqkv, B_wo)
    x = x + _A_ref(_layernorm(x, axis=-1), A_wq, A_wk, A_wv, A_wo)
    x = x + _B_ref(_layernorm(x, axis=-1), B_wqkv, B_wo)
    return x
```

```python
import functools
import jax
import jax.numpy as jnp
from jax import lax
import jax.experimental.pallas as pl
import jax.experimental.pallas.tpu as pltpu

S = 2048
D = 448
H = 16
DH = 28
HP = 32
DP = H * HP
WIN = 256
TC = 512
NCH = S // TC
KC = 256
EPS = 1e-5
LOG2E = 1.4426950408889634
QSCALE = (DH ** -0.5) * LOG2E
L_LO = 2.0 ** -40
BIG = 2.0 ** 100

bf16 = jnp.bfloat16
f32 = jnp.float32


def _dot(a, b):
    return jnp.dot(a, b, preferred_element_type=f32)


def _kernel(x_hbm, wq_hbm, wk_hbm, wv_hbm, wo_hbm, wqkv_hbm, wob_hbm, out_hbm,
            x_in, wq_raw, wk_raw, wv_raw, wo_raw, wqkv_raw, wob_raw,
            tmp, wa_t, wb_t, woa_t, wob_t,
            xt, qx, ka, kb, vta, vtb, ot, bad_ref, sems):
    cp_wq = pltpu.make_async_copy(wq_hbm, wq_raw, sems.at[0])
    cp_wk = pltpu.make_async_copy(wk_hbm, wk_raw, sems.at[1])
    cp_wv = pltpu.make_async_copy(wv_hbm, wv_raw, sems.at[2])
    cp_wo = pltpu.make_async_copy(wo_hbm, wo_raw, sems.at[3])
    cp_wqkv = pltpu.make_async_copy(wqkv_hbm, wqkv_raw, sems.at[4])
    cp_wob = pltpu.make_async_copy(wob_hbm, wob_raw, sems.at[5])

    def x_copy(c):
        return pltpu.make_async_copy(x_hbm.at[:, pl.ds(c * TC, TC)], x_in.at[:, pl.ds(c * TC, TC)], sems.at[6 + c])

    def out_copy(c):
        return pltpu.make_async_copy(x_in.at[:, pl.ds(c * TC, TC)], out_hbm.at[:, pl.ds(c * TC, TC)], sems.at[6 + c])

    cp_wq.start(); cp_wk.start(); cp_wv.start()
    for c in range(NCH):
        x_copy(c).start()
    cp_wo.start(); cp_wqkv.start(); cp_wob.start()

    qx[...] = jnp.zeros(qx.shape, bf16)

    def pad_heads_t(w_t):
        for h in range(H):
            tmp[h * HP:h * HP + DH, :] = w_t[h * DH:(h + 1) * DH, :]
        return tmp[...]

    tmp[...] = jnp.zeros(tmp.shape, f32)
    cp_wk.wait(); cp_wv.wait()
    tmp[0:DH, :] = wk_raw[...].astype(f32)
    tmp[HP:HP + DH, :] = wv_raw[...].astype(f32)
    wa_t[DP:DP + 2 * HP, :] = tmp[0:2 * HP, :].astype(bf16)
    cp_wq.wait()
    wa_t[0:DP, :] = pad_heads_t(wq_raw[...].astype(f32).T).astype(bf16)

    cp_wo.wait()
    woa_t[...] = pad_heads_t(wo_raw[...].astype(f32)).T.astype(bf16)
    cp_wqkv.wait()
    for part in range(3):
        wb_t[part * DP:(part + 1) * DP, :] = pad_heads_t(wqkv_raw[:, part * D:(part + 1) * D].astype(f32).T).astype(bf16)
    cp_wob.wait()
    wob_t[...] = pad_heads_t(wob_raw[...].astype(f32)).T.astype(bf16)

    def layernorm(x):
        m = jnp.mean(x, axis=0, keepdims=True)
        xc = x - m
        v = jnp.mean(xc * xc, axis=0, keepdims=True)
        return (xc * lax.rsqrt(v + EPS)).astype(bf16)

    def store_q(q, c):
        for h in range(H):
            g, j = h // 4, h % 4
            for bb in range(TC // 128):
                col = pl.multiple_of((c * (TC // 128) + bb) * 512 + j * 128, 128)
                qx[g, j * HP:(j + 1) * HP, pl.ds(col, 128)] = (
                    q[h * HP:(h + 1) * HP, bb * 128:(bb + 1) * 128] * QSCALE).astype(bf16)

    def with_ones(v):
        row = lax.broadcasted_iota(jnp.int32, v.shape, 0)
        return jnp.where((row & (HP - 1)) == DH, 1.0, v).astype(bf16)

    def proj_a(x, c):
        tok = pl.ds(pl.multiple_of(c * TC, TC), TC)
        xn = layernorm(x)
        r = _dot(wa_t[...], xn)
        store_q(r[0:DP], c)
        kt = r[DP:DP + HP]
        ka[tok, :] = jnp.concatenate([kt, kt, kt, kt], axis=0).T.astype(bf16)
        vta[:, tok] = with_ones(r[DP + HP:DP + 2 * HP])

    def proj_b(x, c):
        tok = pl.ds(pl.multiple_of(c * TC, TC), TC)
        xn = layernorm(x)
        kt = _dot(wb_t[DP:2 * DP, :], xn)
        for g in range(4):
            kb[g, tok, :] = kt[g * 128:(g + 1) * 128, :].T.astype(bf16)
        q = _dot(wb_t[0:DP, :], xn)
        store_q(q, c)
        v = _dot(wb_t[2 * DP:3 * DP, :], xn)
        vtb[:, tok] = with_ones(v)

    def out_proj(wo_t, c):
        tok = pl.ds(pl.multiple_of(c * TC, TC), TC)
        return xt[:, tok] + _dot(wo_t[...], ot[:, tok])

    def finish(acc, row0, col0, check):
        l = acc[DH:DH + 1, :]
        ot[pl.ds(row0, HP), pl.ds(col0, 128)] = (acc * pl.reciprocal(l, approx=False)).astype(bf16)
        if check:
            ok = jnp.logical_and(jnp.abs(acc) < BIG, l > L_LO)
            return jnp.where(ok, 0.0, 1.0)
        return None

    def attn_a_fast():
        bad_ref[...] = jnp.zeros(bad_ref.shape, f32)

        def body(i, carry):
            g = i // 4
            c = i % 4
            w = qx[g, :, pl.ds(pl.multiple_of(c * 2048, 2048), 2048)]
            acc = None
            for kc in range(S // KC):
                s = _dot(ka[kc * KC:(kc + 1) * KC, :], w)
                p = jnp.exp2(s).astype(bf16)
                pv = _dot(vta[:, kc * KC:(kc + 1) * KC], p)
                acc = pv if acc is None else acc + pv
            bad = bad_ref[...]
            for bb in range(4):
                for j in range(4):
                    n = bb * 4 + j
                    b_ = finish(acc[:, n * 128:(n + 1) * 128],
                                pl.multiple_of((g * 4 + j) * HP, HP),
                                pl.multiple_of((c * 4 + bb) * 128, 128), True)
                    bad = jnp.maximum(bad, b_)
            bad_ref[...] = bad
            return carry

        lax.fori_loop(0, 16, body, 0)

    def attn_a_safe():
        def body(i, carry):
            g = i // 16
            b = i % 16
            w = qx[g, :, pl.ds(pl.multiple_of(b * 512, 512), 512)]
            s = _dot(ka[...], w)
            m = jnp.max(s, axis=0, keepdims=True)
            p = jnp.exp2(s - m).astype(bf16)
            acc = _dot(vta[...], p)
            for j in range(4):
                finish(acc[:, j * 128:(j + 1) * 128], pl.multiple_of((g * 4 + j) * HP, HP),
                       pl.multiple_of(b * 128, 128), False)
            return carry

        lax.fori_loop(0, 64, body, 0)

    def attn_b_fast():
        bad_ref[...] = jnp.zeros(bad_ref.shape, f32)
        krow = lax.broadcasted_iota(jnp.int32, (128, 128), 0)
        qcol = lax.broadcasted_iota(jnp.int32, (128, 128), 1)
        diag = krow <= qcol

        def body(g, carry):
            bad = bad_ref[...]

            def qk(b):
                lo = max(b - 2, 0)
                w = qx[g, :, b * 512:(b + 1) * 512]
                return _dot(kb[g, lo * 128:(b + 1) * 128, :], w)

            s_next = qk(0)
            for b in range(16):
                lo = max(b - 2, 0)
                nk = b + 1 - lo
                s = s_next
                if b + 1 < 16:
                    s_next = qk(b + 1)
                for j in range(4):
                    row0 = pl.multiple_of((g * 4 + j) * HP, HP)
                    sj = s[:, j * 128:(j + 1) * 128]
                    tiles = {lo + t: sj[t * 128:(t + 1) * 128] for t in range(nk)}
                    ps = {}
                    if b >= 2:
                        pc = jnp.exp2(jnp.where(diag, tiles[b], tiles[b - 2]))
                        ps[b] = jnp.where(diag, pc, 0.0)
                        ps[b - 2] = jnp.where(diag, 0.0, pc)
                    else:
                        ps[b] = jnp.where(diag, jnp.exp2(tiles[b]), 0.0)
                    if b >= 1:
                        ps[b - 1] = jnp.exp2(tiles[b - 1])
                    acc = None
                    for t in sorted(ps):
                        pv = _dot(vtb[pl.ds(row0, HP), t * 128:(t + 1) * 128], ps[t].astype(bf16))
                        acc = pv if acc is None else acc + pv
                    bad = jnp.maximum(bad, finish(acc, row0, b * 128, True))
            bad_ref[...] = bad
            return carry

        lax.fori_loop(0, 4, body, 0)

    def attn_b_safe():
        krow = lax.broadcasted_iota(jnp.int32, (384, 512), 0)
        qcol = lax.broadcasted_iota(jnp.int32, (384, 512), 1) & 127

        def body(i, carry):
            g = i // 16
            b = i % 16
            lo = jnp.maximum(b - 2, 0)
            k0 = pl.multiple_of(lo * 128, 128)
            w = qx[g, :, pl.ds(pl.multiple_of(b * 512, 512), 512)]
            s = _dot(kb[g, pl.ds(k0, 384), :], w)
            dist = (b * 128 + qcol) - (k0 + krow)
            valid = jnp.logical_and(dist >= 0, dist < WIN)
            s = jnp.where(valid, s, -1e30)
            m = jnp.max(s, axis=0, keepdims=True)
            p = jnp.where(valid, jnp.exp2(s - m), 0.0).astype(bf16)
            for j in range(4):
                row0 = pl.multiple_of((g * 4 + j) * HP, HP)
                acc = _dot(vtb[pl.ds(row0, HP), pl.ds(k0, 384)], p[:, j * 128:(j + 1) * 128])
                finish(acc, row0, pl.multiple_of(b * 128, 128), False)
            return carry

        lax.fori_loop(0, 64, body, 0)

    def guarded(fast, safe):
        fast()
        unsafe = jnp.max(bad_ref[...]) > 0.0

        @pl.when(unsafe)
        def _():
            safe()

    def first_body(c, carry):
        tok = pl.ds(pl.multiple_of(c * TC, TC), TC)
        x_copy(c).wait()
        x = x_in[:, tok].astype(f32)
        xt[:, tok] = x
        proj_a(x, c)
        return carry

    lax.fori_loop(0, NCH, first_body, 0)

    def mid(wo_t, proj):
        def body(c, carry):
            tok = pl.ds(pl.multiple_of(c * TC, TC), TC)
            x = out_proj(wo_t, c)
            xt[:, tok] = x
            proj(x, c)
            return carry
        lax.fori_loop(0, NCH, body, 0)

    guarded(attn_a_fast, attn_a_safe)
    mid(woa_t, proj_b)
    guarded(attn_b_fast, attn_b_safe)
    mid(wob_t, proj_a)
    guarded(attn_a_fast, attn_a_safe)
    mid(woa_t, proj_b)
    guarded(attn_b_fast, attn_b_safe)

    def last_body(c, carry):
        tok = pl.ds(pl.multiple_of(c * TC, TC), TC)
        x = out_proj(wob_t, c)
        x_in[:, tok] = x.astype(bf16)
        out_copy(c).start()
        return carry

    lax.fori_loop(0, NCH, last_body, 0)
    for c in range(NCH):
        out_copy(c).wait()


@jax.jit
def pallas_interleave_layers__grouped_kv_mqa__sliding_block__prompt_kernel(A_x, A_wq, A_wk, A_wv, A_wo, B_x, B_wqkv, B_wo):
    xt = A_x.reshape(S, D).T
    any_spec = pl.BlockSpec(memory_space=pltpu.HBM)
    out = pl.pallas_call(
        _kernel,
        out_shape=jax.ShapeDtypeStruct((D, S), bf16),
        in_specs=[any_spec] * 7,
        out_specs=any_spec,
        scratch_shapes=[
            pltpu.VMEM((D, S), bf16),
            pltpu.VMEM((D, D), bf16),
            pltpu.VMEM((DH, D), bf16),
            pltpu.VMEM((DH, D), bf16),
            pltpu.VMEM((D, D), bf16),
            pltpu.VMEM((D, 3 * D), bf16),
            pltpu.VMEM((D, D), bf16),
            pltpu.VMEM((DP, D), f32),
            pltpu.VMEM((DP + 2 * HP, D), bf16),
            pltpu.VMEM((3 * DP, D), bf16),
            pltpu.VMEM((D, DP), bf16),
            pltpu.VMEM((D, DP), bf16),
            pltpu.VMEM((D, S), f32),
            pltpu.VMEM((4, 128, 4 * S), bf16),
            pltpu.VMEM((S, 128), bf16),
            pltpu.VMEM((4, S, 128), bf16),
            pltpu.VMEM((HP, S), bf16),
            pltpu.VMEM((DP, S), bf16),
            pltpu.VMEM((DP, S), bf16),
            pltpu.VMEM((HP, 128), f32),
            pltpu.SemaphoreType.DMA((6 + NCH,)),
        ],
        compiler_params=pltpu.CompilerParams(vmem_limit_bytes=100 * 1024 * 1024),
        name="fused_layers",
    )(xt, A_wq, A_wk.T, A_wv.T, A_wo, B_wqkv, B_wo)
    return out.T.reshape(1, S, D)
```

```python
import jax
import jax.numpy as jnp
from jax import lax
import jax.experimental.pallas as pl
import jax.experimental.pallas.tpu as pltpu

S = 2048
D = 448
H = 16
DH = 28
HP = 32
DP = H * HP
GR = 4 * DH
WIN = 256
TC = 512
NCH = S // TC
NB = TC // 128
UT = 2
UB = 2
EPS = 1e-5
LOG2E = 1.4426950408889634
QSCALE = (DH ** -0.5) * LOG2E
L_LO = 2.0 ** -40
L_HI = 2.0 ** 60
V_HI = 2.0 ** 60
OC = 256
NVS = (96, 80)
NV = max(NVS)
NPAIR = 0
LEAD = 2
QW = 256
STAGED = (0, 8)
DIRECT = [t for t in range(16) if t not in STAGED]

bf16 = jnp.bfloat16
f32 = jnp.float32
u32 = jnp.uint32


def _dot(a, b):
    return jnp.dot(a, b, preferred_element_type=f32)


def _dot_tn(a, b):
    return lax.dot_general(a, b, (((0,), (0,)), ((), ())), preferred_element_type=f32)


def _kernel(x_hbm, wq_hbm, wk_hbm, wv_hbm, wo_hbm, wqkv_hbm, wob_hbm, out_hbm,
            x_in, wq, wk_raw, wv_raw, woa, wqkv, wob,
            wkv, woat, wobt, xt, qd, qf, qx, ka, kbc, kb, vta, vtb, ot, pbuf, accbuf, lmin_ref, lmax_ref, vmax_ref, sems):
    cp_wq = pltpu.make_async_copy(wq_hbm, wq, sems.at[0])
    cp_wk = pltpu.make_async_copy(wk_hbm, wk_raw, sems.at[1])
    cp_wv = pltpu.make_async_copy(wv_hbm, wv_raw, sems.at[2])
    cp_wo = pltpu.make_async_copy(wo_hbm, woa, sems.at[3])
    cp_wqkv = pltpu.make_async_copy(wqkv_hbm, wqkv, sems.at[4])
    cp_wob = pltpu.make_async_copy(wob_hbm, wob, sems.at[5])

    def x_copy(c):
        return pltpu.make_async_copy(x_hbm.at[:, pl.ds(c * TC, TC)], x_in.at[:, pl.ds(c * TC, TC)], sems.at[6 + c])

    def out_copy(c):
        return pltpu.make_async_copy(x_in.at[:, pl.ds(c * OC, OC)], out_hbm.at[:, pl.ds(c * OC, OC)], sems.at[6 + NCH + c])

    x_copy(0).start()
    cp_wk.start(); cp_wv.start(); cp_wq.start()
    x_copy(1).start()

    def slab(j):
        return (j * DH) // 16 * 16, -(-(j * DH + DH) // 16) * 16

    qx[...] = jnp.zeros(qx.shape, bf16)
    pbuf[...] = jnp.zeros(pbuf.shape, bf16)
    accbuf[...] = jnp.ones(accbuf.shape, f32)
    vmax_ref[...] = jnp.zeros(vmax_ref.shape, f32)

    cp_wk.wait(); cp_wv.wait()
    zpad = jnp.zeros((HP - DH, D), f32)
    wkv[...] = jnp.concatenate([wk_raw[...].astype(f32), zpad, wv_raw[...].astype(f32), zpad], axis=0).astype(bf16)
    cp_wq.wait()
    for c in range(2, NCH):
        x_copy(c).start()
    cp_wo.start(); cp_wob.start(); cp_wqkv.start()

    def layernorm(x):
        outs = []
        for t in range(x.shape[1] // 128):
            xs = x[:, t * 128:(t + 1) * 128]
            m = jnp.mean(xs, axis=0, keepdims=True)
            xc = xs - m
            v = jnp.mean(xc * xc, axis=0, keepdims=True)
            outs.append(xc * lax.rsqrt(v + EPS))
        return jnp.concatenate(outs, axis=1).astype(bf16)

    def v_slab(v):
        row = lax.broadcasted_iota(jnp.int32, v.shape, 0)
        return jnp.where(row < DH, v, jnp.where(row == DH, 1.0, 0.0)).astype(bf16)

    def track_v(v):
        m = vmax_ref[...]
        a = jnp.abs(v)
        for r in range(0, v.shape[0], 8):
            for c0 in range(0, v.shape[1], 128):
                m = jnp.maximum(m, a[r:r + 8, c0:c0 + 128])
        vmax_ref[...] = m

    def proj_a(x, it, u, qsplit=0):
        c = it * UT + u
        tok = pl.ds(pl.multiple_of(c * TC, TC), TC)
        xn = layernorm(x)
        parts = []
        if qsplit > 0:
            parts.append(_dot_tn(wq[...], xn[:, 0:qsplit]))
        kv = _dot(wkv[...], xn)
        if qsplit < TC:
            parts.append(_dot_tn(wq[...], xn[:, qsplit:TC]))
        q = parts[0] if len(parts) == 1 else jnp.concatenate(parts, axis=1)
        q = q * QSCALE
        kt = kv[0:HP]
        kn = jnp.concatenate([kt, kt, kt, kt], axis=0).T
        ka[tok, :] = kn.astype(bf16)
        if u == 0:
            rows = pl.ds(pl.multiple_of(it * NV, 8), NV)
            for d in range(DH):
                kbc[d, rows, :] = jnp.broadcast_to(kn[0:NV, d:d + 1], (NV, 128))
        vta[:, tok] = v_slab(kv[HP:2 * HP])
        track_v(kv[HP:2 * HP])
        for g in range(4):
            for k in range(TC // QW):
                qf[g, c * (TC // QW) + k] = q[g * GR:(g + 1) * GR, k * QW:(k + 1) * QW]
        q = jnp.concatenate([q, q[0:8]], axis=0)
        for g in range(4):
            for bb in range(NB):
                col = pl.ds(pl.multiple_of((c * NB + bb) * 512, 512), 512)
                qd[g, :, col] = jnp.concatenate(
                    [q[(g * 4 + j) * DH:(g * 4 + j) * DH + HP, bb * 128:(bb + 1) * 128] for j in range(4)],
                    axis=1).astype(bf16)

    def proj_b(x, it, u):
        c = it * UT + u
        tok = pl.ds(pl.multiple_of(c * TC, TC), TC)
        xn = layernorm(x)
        kt = _dot_tn(wqkv[:, D:2 * D], xn)
        kt = jnp.concatenate([kt, kt[0:16]], axis=0)
        for g in range(4):
            kb[g, tok, :] = kt[g * GR:g * GR + 128, :].T.astype(bf16)
        q = _dot_tn(wqkv[:, 0:D], xn) * QSCALE
        for h in range(H):
            g, j = h // 4, h % 4
            r0, r1 = slab(j)
            row = lax.broadcasted_iota(jnp.int32, (r1 - r0, 128), 0) + r0
            keep = jnp.logical_and(row >= j * DH, row < (j + 1) * DH)
            for bb in range(NB):
                col = pl.multiple_of((c * NB + bb) * 512 + j * 128, 128)
                piece = q[g * GR + r0:g * GR + r1, bb * 128:(bb + 1) * 128]
                qx[g, r0:r1, pl.ds(col, 128)] = jnp.where(keep, piece, 0.0).astype(bf16)
        v = _dot_tn(wqkv[:, 2 * D:3 * D], xn)
        track_v(v)
        v = jnp.concatenate([v, v[0:8]], axis=0)
        for h in range(H):
            vtb[h * HP:(h + 1) * HP, tok] = v_slab(v[h * DH:h * DH + HP, :])

    def out_proj(wo, c, src):
        tok = pl.ds(pl.multiple_of(c * TC, TC), TC)
        return src[:, tok].astype(f32) + _dot(pltpu.bitcast(wo[...], bf16), ot[:, tok])

    def q_tiles(q_ref, g, b, n):
        start = b * 512 if isinstance(b, int) else pl.multiple_of(b * 512, 512)
        return q_ref[g, :, pl.ds(start, 512 * n)]

    def finish(accs, g, col0, stat):
        outs = []
        for acc in accs:
            l = acc[DH:DH + 1, :]
            r = pl.reciprocal(l, approx=True)
            r = r * (2.0 - l * r)
            outs.append(acc[0:DH, :] * r)
            if stat is not None:
                stat = (jnp.minimum(stat[0], acc[24:32, :]), jnp.maximum(stat[1], acc[24:32, :]))
        ot[pl.ds(pl.multiple_of(g * GR, 16), GR), pl.ds(col0, 128)] = jnp.concatenate(outs, axis=0).astype(bf16)
        return stat

    def reset_stat():
        lmin_ref[...] = jnp.ones(lmin_ref.shape, f32)
        lmax_ref[...] = jnp.ones(lmax_ref.shape, f32)

    def tiles_k(ts):
        parts = [ka[t * 128:(t + 1) * 128, 0:HP] for t in ts]
        return parts[0] if len(parts) == 1 else jnp.concatenate(parts, axis=0)

    def tiles_v(ts):
        parts = [vta[:, t * 128:(t + 1) * 128] for t in ts]
        return parts[0] if len(parts) == 1 else jnp.concatenate(parts, axis=1)

    d_groups = []
    d0 = 0
    for t in range(DH - NPAIR):
        two = ((t + 1) * NPAIR) // (DH - NPAIR) - (t * NPAIR) // (DH - NPAIR)
        d_groups.append(list(range(d0, d0 + 1 + two)))
        d0 += 1 + two

    def attn_a_fast():
        reset_stat()

        def staged_pv(n):
            return accbuf[:, n * 128:(n + 1) * 128] + _dot(tiles_v(STAGED), pbuf[n])

        def body(i, carry):
            g = i // 4
            c = i % 4
            ip = jnp.maximum(i - 1, 0)
            gp = ip // 4
            cp = ip % 4
            stat0 = (lmin_ref[...], lmax_ref[...])
            never = stat0[0] > stat0[1]
            state = {'link': None, 'stat': stat0, 'done': []}

            def finish_prev(n):
                state['done'].append(staged_pv(n))
                if len(state['done']) == 4:
                    state['stat'] = finish(state['done'], gp, pl.multiple_of((cp * 4 + n // 4) * 128, 128), state['stat'])
                    state['done'] = []

            def vpu_job(n, k, r):
                bb, j = n // 4, n % 4
                k0 = k * NV + r * 16
                qcols = pl.ds((bb * 128) % QW, 128)
                a = [None, None]
                for grp in d_groups:
                    ts = [None, None]
                    for d in grp:
                        qrow = jnp.broadcast_to(
                            qf[g, c * (512 // QW) + (bb * 128) // QW, j * DH + d:j * DH + d + 1, qcols], (8, 128))
                        for v in range(2):
                            t = kbc[d, k0 + v * 8:k0 + v * 8 + 8, :] * qrow
                            ts[v] = t if ts[v] is None else ts[v] + t
                    for v in range(2):
                        if a[v] is None:
                            a[v] = ts[v] if state['link'] is None else jnp.where(never, state['link'][1 - v], ts[v])
                        else:
                            a[v] = a[v] + ts[v]
                state['link'] = a
                row = k * 128 + r * 16
                pbuf[n, row:row + 16, :] = jnp.exp2(jnp.concatenate(a, axis=0)).astype(bf16)

            jobs = [(n, k, r) for n in range(16) for k in range(2) for r in range(NVS[k] // 16)]
            chunks = [DIRECT[k:k + 2] for k in range(0, len(DIRECT), 2)]
            steps = [(qb, ch) for qb in range(4) for ch in chunks]
            accs = {}
            pend = []

            def pv(qb, ch, s):
                r = _dot(tiles_v(ch), jnp.exp2(s).astype(bf16))
                accs[qb] = r if qb not in accs else accs[qb] + r

            ji = 0
            po = 0
            for t, (qb, ch) in enumerate(steps):
                target = ((t + 1) * len(jobs)) // len(steps)
                need = min(16, (jobs[target - 1][0] if target else 0) + 1 + LEAD)
                while po < need:
                    finish_prev(po)
                    po += 1
                w = q_tiles(qd, g, c * 4 + qb, 1)
                pend.append((qb, ch, _dot(tiles_k(ch), w)))
                while ji < target:
                    vpu_job(*jobs[ji])
                    ji += 1
                if t == len(steps) - 1:
                    krest = jnp.concatenate(
                        [ka[st * 128 + NVS[k]:(st + 1) * 128, 0:HP] for k, st in enumerate(STAGED)], axis=0)
                    p = jnp.exp2(_dot(krest, q_tiles(qd, g, c * 4, 4)))
                    for n in range(16):
                        for k in range(2):
                            r0 = k * (128 - NVS[0])
                            pbuf[n, k * 128 + NVS[k]:(k + 1) * 128, :] = (
                                p[r0:r0 + 128 - NVS[k], n * 128:(n + 1) * 128].astype(bf16))
                if len(pend) > 1:
                    pv(*pend.pop(0))
            while pend:
                pv(*pend.pop(0))
            for qb in range(4):
                accbuf[:, qb * 512:(qb + 1) * 512] = accs[qb]
            lmin_ref[...] = jnp.where(i > 0, state['stat'][0], stat0[0])
            lmax_ref[...] = jnp.where(i > 0, state['stat'][1], stat0[1])
            return carry

        lax.fori_loop(0, 16, body, 0)
        stat = (lmin_ref[...], lmax_ref[...])
        for bb in range(4):
            stat = finish([staged_pv(bb * 4 + j) for j in range(4)], 3, (12 + bb) * 128, stat)
        lmin_ref[...] = stat[0]
        lmax_ref[...] = stat[1]

    def attn_a_safe():
        def body(i, carry):
            g = i // 16
            b = i % 16
            w = q_tiles(qd, g, b, 1)
            s = _dot(ka[:, 0:HP], w)
            m = jnp.max(s, axis=0, keepdims=True)
            p = jnp.exp2(s - m).astype(bf16)
            acc = _dot(vta[...], p)
            finish([acc[:, j * 128:(j + 1) * 128] for j in range(4)], g, pl.multiple_of(b * 128, 128), None)
            return carry

        lax.fori_loop(0, 64, body, 0)

    def attn_b_fast():
        reset_stat()
        krow = lax.broadcasted_iota(jnp.int32, (128, 128), 0)
        qcol = lax.broadcasted_iota(jnp.int32, (128, 128), 1)
        diag = krow <= qcol

        def body(it, carry):
            stat = (lmin_ref[...], lmax_ref[...])

            def qk(g, b):
                lo = max(b - 2, 0)
                w = q_tiles(qx, g, b, 1)
                return _dot(kb[g, lo * 128:(b + 1) * 128, :], w)

            items = [(it * UB + u, b) for u in range(UB) for b in range(16)]
            s_next = qk(*items[0])
            for n, (g, b) in enumerate(items):
                lo = max(b - 2, 0)
                nk = b + 1 - lo
                s = s_next
                if n + 1 < len(items):
                    s_next = qk(*items[n + 1])
                accs = []
                for j in range(4):
                    row0 = pl.multiple_of((g * 4 + j) * HP, HP)
                    sj = s[:, j * 128:(j + 1) * 128]
                    tiles = {lo + t: sj[t * 128:(t + 1) * 128] for t in range(nk)}
                    ps = {}
                    if b >= 2:
                        pc = jnp.exp2(jnp.where(diag, tiles[b], tiles[b - 2]))
                        ps[b] = jnp.where(diag, pc, 0.0)
                        ps[b - 2] = jnp.where(diag, 0.0, pc)
                    else:
                        ps[b] = jnp.where(diag, jnp.exp2(tiles[b]), 0.0)
                    if b >= 1:
                        ps[b - 1] = jnp.exp2(tiles[b - 1])
                    acc = None
                    for t in sorted(ps):
                        pv = _dot(vtb[pl.ds(row0, HP), t * 128:(t + 1) * 128], ps[t].astype(bf16))
                        acc = pv if acc is None else acc + pv
                    accs.append(acc)
                stat = finish(accs, g, b * 128, stat)
            lmin_ref[...] = stat[0]
            lmax_ref[...] = stat[1]
            return carry

        lax.fori_loop(0, 4 // UB, body, 0)

    def attn_b_safe():
        krow = lax.broadcasted_iota(jnp.int32, (384, 512), 0)
        qcol = lax.broadcasted_iota(jnp.int32, (384, 512), 1) & 127

        def body(i, carry):
            g = i // 16
            b = i % 16
            lo = jnp.maximum(b - 2, 0)
            k0 = pl.multiple_of(lo * 128, 128)
            w = q_tiles(qx, g, b, 1)
            s = _dot(kb[g, pl.ds(k0, 384), :], w)
            dist = (b * 128 + qcol) - (k0 + krow)
            valid = jnp.logical_and(dist >= 0, dist < WIN)
            s = jnp.where(valid, s, -1e30)
            m = jnp.max(s, axis=0, keepdims=True)
            p = jnp.where(valid, jnp.exp2(s - m), 0.0).astype(bf16)
            accs = []
            for j in range(4):
                row0 = pl.multiple_of((g * 4 + j) * HP, HP)
                accs.append(_dot(vtb[pl.ds(row0, HP), pl.ds(k0, 384)], p[:, j * 128:(j + 1) * 128]))
            finish(accs, g, pl.multiple_of(b * 128, 128), None)
            return carry

        lax.fori_loop(0, 64, body, 0)

    def guarded(fast, safe):
        fast()
        row = lax.broadcasted_iota(jnp.int32, (8, 128), 0)
        l_ok = jnp.logical_and(lmin_ref[...] > L_LO, lmax_ref[...] < L_HI)
        ok = jnp.logical_and(jnp.logical_or(l_ok, row != DH - 24), vmax_ref[...] < V_HI)
        unsafe = jnp.max(jnp.where(ok, 0.0, 1.0)) > 0.0

        @pl.when(unsafe)
        def _():
            safe()

    def first_body(it, carry):
        for u in range(UT):
            x_copy(it * UT + u).wait()
        for u in range(UT):
            c = it * UT + u
            tok = pl.ds(pl.multiple_of(c * TC, TC), TC)
            proj_a(x_in[:, tok].astype(f32), it, u, (512, 384)[u])
        return carry

    lax.fori_loop(0, NCH // UT, first_body, 0)
    cp_wo.wait(); cp_wob.wait()
    woat[...] = pltpu.bitcast(woa[...].T, u32)
    wobt[...] = pltpu.bitcast(wob[...].T, u32)

    def mid(wo, proj, src):
        def body(it, carry):
            x_next = out_proj(wo, it * UT, src)
            for u in range(UT):
                c = it * UT + u
                tok = pl.ds(pl.multiple_of(c * TC, TC), TC)
                x = x_next
                if u + 1 < UT:
                    x_next = out_proj(wo, c + 1, src)
                xt[:, tok] = x
                proj(x, it, u)
            return carry
        lax.fori_loop(0, NCH // UT, body, 0)

    guarded(attn_a_fast, attn_a_safe)
    cp_wqkv.wait()
    mid(woat, proj_b, x_in)
    guarded(attn_b_fast, attn_b_safe)
    mid(wobt, proj_a, xt)
    guarded(attn_a_fast, attn_a_safe)
    mid(woat, proj_b, xt)
    guarded(attn_b_fast, attn_b_safe)

    def last_body(it, carry):
        xs = [out_proj(wobt, it * UT + u, xt) for u in range(UT)]
        for u in range(UT):
            for k in range(TC // OC):
                c = (it * UT + u) * (TC // OC) + k
                x_in[:, pl.ds(pl.multiple_of(c * OC, OC), OC)] = xs[u][:, k * OC:(k + 1) * OC].astype(bf16)
                out_copy(c).start()
        return carry

    lax.fori_loop(0, NCH // UT, last_body, 0)
    for c in range(S // OC):
        out_copy(c).wait()


@jax.jit
def pallas_interleave_layers__grouped_kv_mqa__sliding_block__prompt_kernel(A_x, A_wq, A_wk, A_wv, A_wo, B_x, B_wqkv, B_wo):
    xt = A_x.reshape(S, D).T
    hbm_spec = pl.BlockSpec(memory_space=pltpu.HBM)
    out = pl.pallas_call(
        _kernel,
        out_shape=jax.ShapeDtypeStruct((D, S), bf16),
        in_specs=[hbm_spec] * 7,
        out_specs=hbm_spec,
        scratch_shapes=[
            pltpu.VMEM((D, S), bf16),
            pltpu.VMEM((D, D), bf16),
            pltpu.VMEM((DH, D), bf16),
            pltpu.VMEM((DH, D), bf16),
            pltpu.VMEM((D, D), bf16),
            pltpu.VMEM((D, 3 * D), bf16),
            pltpu.VMEM((D, D), bf16),
            pltpu.VMEM((2 * HP, D), bf16),
            pltpu.VMEM((D // 2, D), u32),
            pltpu.VMEM((D // 2, D), u32),
            pltpu.VMEM((D, S), f32),
            pltpu.VMEM((4, HP, 4 * S), bf16),
            pltpu.VMEM((4, S // QW, GR, QW), f32),
            pltpu.VMEM((4, 128, 4 * S), bf16),
            pltpu.VMEM((S, 128), bf16),
            pltpu.VMEM((DH, 2 * NV, 128), f32),
            pltpu.VMEM((4, S, 128), bf16),
            pltpu.VMEM((HP, S), bf16),
            pltpu.VMEM((DP, S), bf16),
            pltpu.VMEM((D, S), bf16),
            pltpu.VMEM((16, 256, 128), bf16),
            pltpu.VMEM((HP, S), f32),
            pltpu.VMEM((8, 128), f32),
            pltpu.VMEM((8, 128), f32),
            pltpu.VMEM((8, 128), f32),
            pltpu.SemaphoreType.DMA((6 + NCH + S // OC,)),
        ],
        compiler_params=pltpu.CompilerParams(vmem_limit_bytes=100 * 1024 * 1024),
        name="fused_layers",
    )(xt, A_wq, A_wk.T, A_wv.T, A_wo, B_wqkv, B_wo)
    return out.T.reshape(1, S, D)
```

```python
import jax
import jax.numpy as jnp
from jax import lax
import jax.experimental.pallas as pl
import jax.experimental.pallas.tpu as pltpu

S = 2048
D = 448
H = 16
DH = 28
HP = 32
DP = H * HP
GR = 4 * DH
WIN = 256
TC = 512
TF = 256
UT = 1024 // TC
NB = TC // 128
UB = 2
OC = 128
QW = 256
EPS = 1e-5
LOG2E = 1.4426950408889634
QSCALE = (DH ** -0.5) * LOG2E
L_LO = 2.0 ** -40
L_HI = 2.0 ** 60
V_HI = 2.0 ** 60
STAGED = (0, 8)
NVS = (96, 80)
NV = max(NVS)
LEAD = 2
DIRECT = [t for t in range(16) if t not in STAGED]

bf16 = jnp.bfloat16
f32 = jnp.float32
u32 = jnp.uint32


def _dot(a, b):
    return jnp.dot(a, b, preferred_element_type=f32)


def _dot_tn(a, b):
    return lax.dot_general(a, b, (((0,), (0,)), ((), ())), preferred_element_type=f32)


def _slab(j):
    return (j * DH) // 16 * 16, -(-(j * DH + DH) // 16) * 16


def _kernel(x_hbm, wq_hbm, wk_hbm, wv_hbm, wo_hbm, wqkv_hbm, wob_hbm, out_hbm,
            x_in, wq, wk_raw, wv_raw, woa, wqkv, wob,
            wat, woat, wobt, xa, xb, o_stage, qd, qf, qx, ka, kbc, kb, vta, vtb, ot, pbuf, accbuf,
            lmin_ref, lmax_ref, vmax_ref, flag, sems):
    cp_wq = pltpu.make_async_copy(wq_hbm, wq, sems.at[0])
    cp_wk = pltpu.make_async_copy(wk_hbm, wk_raw, sems.at[1])
    cp_wv = pltpu.make_async_copy(wv_hbm, wv_raw, sems.at[2])
    cp_wo = pltpu.make_async_copy(wo_hbm, woa, sems.at[3])
    cp_wqkv = pltpu.make_async_copy(wqkv_hbm, wqkv, sems.at[4])
    cp_wob = pltpu.make_async_copy(wob_hbm, wob, sems.at[5])

    def x_copy(c):
        return pltpu.make_async_copy(x_hbm.at[:, pl.ds(c * 512, 512)], x_in.at[:, pl.ds(c * 512, 512)],
                                     sems.at[6 + c])

    def out_copy(c):
        return pltpu.make_async_copy(o_stage.at[:, pl.ds(c * OC, OC)], out_hbm.at[:, pl.ds(c * OC, OC)],
                                     sems.at[10 + c])

    x_copy(0).start()
    cp_wk.start()
    cp_wv.start()
    cp_wq.start()
    x_copy(1).start()

    qx[...] = jnp.zeros(qx.shape, bf16)
    pbuf[...] = jnp.zeros(pbuf.shape, bf16)
    accbuf[...] = jnp.ones(accbuf.shape, f32)
    vmax_ref[...] = jnp.zeros(vmax_ref.shape, f32)
    lmin_ref[...] = jnp.ones(lmin_ref.shape, f32)
    lmax_ref[...] = jnp.ones(lmax_ref.shape, f32)

    cp_wk.wait()
    cp_wv.wait()
    zpad = jnp.zeros((HP - DH, D), f32)
    wat[0:HP, :] = pltpu.bitcast(
        jnp.concatenate([wk_raw[...].astype(f32), zpad, wv_raw[...].astype(f32), zpad], axis=0).astype(bf16), u32)
    cp_wq.wait()
    wat[HP:HP + D // 2, :] = pltpu.bitcast(wq[...].T, u32)
    x_copy(0).wait()
    x_copy(1).wait()
    x_copy(2).start()
    x_copy(3).start()
    cp_wo.start()
    cp_wob.start()
    flag[0] = 1

    def layernorm(x):
        outs = []
        for t in range(x.shape[1] // 128):
            xs = x[:, t * 128:(t + 1) * 128]
            m = jnp.mean(xs, axis=0, keepdims=True)
            xc = xs - m
            v = jnp.mean(xc * xc, axis=0, keepdims=True)
            outs.append(xc * lax.rsqrt(v + EPS))
        return jnp.concatenate(outs, axis=1).astype(bf16)

    def v_slab(v):
        row = lax.broadcasted_iota(jnp.int32, v.shape, 0)
        return jnp.where(row < DH, v, jnp.where(row == DH, 1.0, 0.0)).astype(bf16)

    def track_v(v):
        m = vmax_ref[...]
        a = jnp.abs(v)
        for r in range(0, v.shape[0], 8):
            for c0 in range(0, v.shape[1], 128):
                m = jnp.maximum(m, a[r:r + 8, c0:c0 + 128])
        vmax_ref[...] = m

    def proj_a(x, it, u, tc=TC):
        c = it * (1024 // tc) + u
        nb = tc // 128
        tok = pl.ds(pl.multiple_of(c * tc, tc), tc)
        kvq = _dot(pltpu.bitcast(wat[...], bf16), layernorm(x))
        q = kvq[2 * HP:] * QSCALE
        kt = kvq[0:HP]
        kn = jnp.concatenate([kt, kt, kt, kt], axis=0).T
        ka[tok, :] = kn.astype(bf16)
        if u == 0:
            rows = pl.ds(pl.multiple_of(it * NV, 8), NV)
            for d in range(DH):
                kbc[d, rows, :] = jnp.broadcast_to(kn[0:NV, d:d + 1], (NV, 128))
        vta[:, tok] = v_slab(kvq[HP:2 * HP])
        track_v(kvq[HP:2 * HP])
        for g in range(4):
            for k in range(tc // QW):
                qf[g, c * (tc // QW) + k] = q[g * GR:(g + 1) * GR, k * QW:(k + 1) * QW]
        q = jnp.concatenate([q, q[0:8]], axis=0)
        for g in range(4):
            for bb in range(nb):
                col = pl.ds(pl.multiple_of((c * nb + bb) * 512, 512), 512)
                qd[g, :, col] = jnp.concatenate(
                    [q[(g * 4 + j) * DH:(g * 4 + j) * DH + HP, bb * 128:(bb + 1) * 128] for j in range(4)],
                    axis=1).astype(bf16)

    def proj_b(x, it, u):
        c = it * UT + u
        tok = pl.ds(pl.multiple_of(c * TC, TC), TC)
        xn = layernorm(x)
        kt = _dot_tn(wqkv[:, D:2 * D], xn)
        kt = jnp.concatenate([kt, kt[0:16]], axis=0)
        for g in range(4):
            kb[g, tok, :] = kt[g * GR:g * GR + 128, :].T.astype(bf16)
        q = _dot_tn(wqkv[:, 0:D], xn) * QSCALE
        for h in range(H):
            g, j = h // 4, h % 4
            r0, r1 = _slab(j)
            row = lax.broadcasted_iota(jnp.int32, (r1 - r0, 128), 0) + r0
            keep = jnp.logical_and(row >= j * DH, row < (j + 1) * DH)
            for bb in range(NB):
                col = pl.multiple_of((c * NB + bb) * 512 + j * 128, 128)
                piece = q[g * GR + r0:g * GR + r1, bb * 128:(bb + 1) * 128]
                qx[g, r0:r1, pl.ds(col, 128)] = jnp.where(keep, piece, 0.0).astype(bf16)
        v = _dot_tn(wqkv[:, 2 * D:3 * D], xn)
        track_v(v)
        v = jnp.concatenate([v, v[0:8]], axis=0)
        for h in range(H):
            vtb[h * HP:(h + 1) * HP, tok] = v_slab(v[h * DH:h * DH + HP, :])

    def out_proj(wo_t, c, src):
        tok = pl.ds(pl.multiple_of(c * TC, TC), TC)
        return src[:, tok] + _dot(pltpu.bitcast(wo_t[...], bf16), ot[:, tok])

    def q_tiles(q_ref, g, b, n):
        start = b * 512 if isinstance(b, int) else pl.multiple_of(b * 512, 512)
        return q_ref[g, :, pl.ds(start, 512 * n)]

    def finish(accs, g, col0, stat):
        outs = []
        for acc in accs:
            l = acc[DH:DH + 1, :]
            r = pl.reciprocal(l, approx=True)
            r = r * (2.0 - l * r)
            outs.append(acc[0:DH, :] * r)
            if stat is not None:
                stat = (jnp.minimum(stat[0], acc[24:32, :]), jnp.maximum(stat[1], acc[24:32, :]))
        ot[pl.ds(pl.multiple_of(g * GR, 16), GR), pl.ds(col0, 128)] = jnp.concatenate(outs, axis=0).astype(bf16)
        return stat

    def tiles_k(ts):
        return jnp.concatenate([ka[t * 128:(t + 1) * 128, 0:HP] for t in ts], axis=0)

    def tiles_v(ts):
        return jnp.concatenate([vta[:, t * 128:(t + 1) * 128] for t in ts], axis=1)

    def attn_a_fast():
        def staged_pv(n):
            return accbuf[:, n * 128:(n + 1) * 128] + _dot(tiles_v(STAGED), pbuf[n])

        def body(i, carry):
            g = i // 4
            c = i % 4
            ip = jnp.maximum(i - 1, 0)
            gp = ip // 4
            cp = ip % 4
            stat0 = (lmin_ref[...], lmax_ref[...])
            never = stat0[0] > stat0[1]
            state = {'link': None, 'stat': stat0, 'done': []}

            def finish_prev(n):
                state['done'].append(staged_pv(n))
                if len(state['done']) == 4:
                    col0 = pl.multiple_of((cp * 4 + n // 4) * 128, 128)
                    state['stat'] = finish(state['done'], gp, col0, state['stat'])
                    state['done'] = []

            def vpu_job(n, k, r):
                bb, j = n // 4, n % 4
                k0 = k * NV + r * 16
                qblk = c * (512 // QW) + (bb * 128) // QW
                qcols = pl.ds((bb * 128) % QW, 128)
                a = None
                for d in range(DH):
                    t = kbc[d, k0:k0 + 16, :] * qf[g, qblk, j * DH + d:j * DH + d + 1, qcols]
                    if a is not None:
                        a = a + t
                    elif state['link'] is None:
                        a = t
                    else:
                        lk = state['link']
                        a = jnp.concatenate(
                            [jnp.where(never, lk[8:16], t[0:8]), jnp.where(never, lk[0:8], t[8:16])], axis=0)
                state['link'] = a
                row = k * 128 + r * 16
                pbuf[n, row:row + 16, :] = jnp.exp2(a).astype(bf16)

            jobs = [(n, k, r) for n in range(16) for k in range(2) for r in range(NVS[k] // 16)]
            chunks = [DIRECT[k:k + 2] for k in range(0, len(DIRECT), 2)]
            steps = [(qb, ch) for qb in range(4) for ch in chunks]
            accs = {}
            pend = []

            def pv(qb, ch, s):
                r = _dot(tiles_v(ch), jnp.exp2(s).astype(bf16))
                accs[qb] = r if qb not in accs else accs[qb] + r

            ji = 0
            po = 0
            for t, (qb, ch) in enumerate(steps):
                target = ((t + 1) * len(jobs)) // len(steps)
                need = min(16, jobs[target - 1][0] + 1 + LEAD)
                while po < need:
                    finish_prev(po)
                    po += 1
                pend.append((qb, ch, _dot(tiles_k(ch), q_tiles(qd, g, c * 4 + qb, 1))))
                while ji < target:
                    vpu_job(*jobs[ji])
                    ji += 1
                if t == len(steps) - 1:
                    krest = jnp.concatenate(
                        [ka[st * 128 + NVS[k]:(st + 1) * 128, 0:HP] for k, st in enumerate(STAGED)], axis=0)
                    p = jnp.exp2(_dot(krest, q_tiles(qd, g, c * 4, 4)))
                    for n in range(16):
                        for k in range(2):
                            r0 = k * (128 - NVS[0])
                            pbuf[n, k * 128 + NVS[k]:(k + 1) * 128, :] = (
                                p[r0:r0 + 128 - NVS[k], n * 128:(n + 1) * 128].astype(bf16))
                if len(pend) > 1:
                    pv(*pend.pop(0))
            while pend:
                pv(*pend.pop(0))
            for qb in range(4):
                accbuf[:, qb * 512:(qb + 1) * 512] = accs[qb]
            lmin_ref[...] = jnp.where(i > 0, state['stat'][0], stat0[0])
            lmax_ref[...] = jnp.where(i > 0, state['stat'][1], stat0[1])
            return carry

        lax.fori_loop(0, 16, body, 0)
        woat[...] = pltpu.bitcast(woa[...].T, u32)
        stat = (lmin_ref[...], lmax_ref[...])
        for bb in range(4):
            stat = finish([staged_pv(bb * 4 + j) for j in range(4)], 3, (12 + bb) * 128, stat)
        lmin_ref[...] = stat[0]
        lmax_ref[...] = stat[1]

    def attn_a_safe():
        def body(i, carry):
            g = i // 16
            b = i % 16
            s = _dot(ka[:, 0:HP], q_tiles(qd, g, b, 1))
            m = jnp.max(s, axis=0, keepdims=True)
            p = jnp.exp2(s - m).astype(bf16)
            acc = _dot(vta[...], p)
            finish([acc[:, j * 128:(j + 1) * 128] for j in range(4)], g, pl.multiple_of(b * 128, 128), None)
            return carry

        lax.fori_loop(0, 64, body, 0)

    def attn_b_fast():
        krow = lax.broadcasted_iota(jnp.int32, (128, 128), 0)
        qcol = lax.broadcasted_iota(jnp.int32, (128, 128), 1)
        diag = krow <= qcol

        def body(it, carry):
            stat = (lmin_ref[...], lmax_ref[...])

            def qk(g, b):
                lo = max(b - 2, 0)
                return _dot(kb[g, lo * 128:(b + 1) * 128, :], q_tiles(qx, g, b, 1))

            items = [(it * UB + u, b) for u in range(UB) for b in range(16)]
            s_next = qk(*items[0])
            for n, (g, b) in enumerate(items):
                lo = max(b - 2, 0)
                nk = b + 1 - lo
                s = s_next
                if n + 1 < len(items):
                    s_next = qk(*items[n + 1])
                accs = []
                for j in range(4):
                    row0 = pl.multiple_of((g * 4 + j) * HP, HP)
                    sj = s[:, j * 128:(j + 1) * 128]
                    tiles = {lo + t: sj[t * 128:(t + 1) * 128] for t in range(nk)}
                    ps = {}
                    if b >= 2:
                        pc = jnp.exp2(jnp.where(diag, tiles[b], tiles[b - 2]))
                        ps[b] = jnp.where(diag, pc, 0.0)
                        ps[b - 2] = jnp.where(diag, 0.0, pc)
                    else:
                        ps[b] = jnp.where(diag, jnp.exp2(tiles[b]), 0.0)
                    if b >= 1:
                        ps[b - 1] = jnp.exp2(tiles[b - 1])
                    acc = None
                    for t in sorted(ps):
                        pv = _dot(vtb[pl.ds(row0, HP), t * 128:(t + 1) * 128], ps[t].astype(bf16))
                        acc = pv if acc is None else acc + pv
                    accs.append(acc)
                stat = finish(accs, g, b * 128, stat)
            lmin_ref[...] = stat[0]
            lmax_ref[...] = stat[1]
            return carry

        lax.fori_loop(0, 4 // UB, body, 0)

    def attn_b_safe():
        krow = lax.broadcasted_iota(jnp.int32, (384, 512), 0)
        qcol = lax.broadcasted_iota(jnp.int32, (384, 512), 1) & 127

        def body(i, carry):
            g = i // 16
            b = i % 16
            k0 = pl.multiple_of(jnp.maximum(b - 2, 0) * 128, 128)
            s = _dot(kb[g, pl.ds(k0, 384), :], q_tiles(qx, g, b, 1))
            dist = (b * 128 + qcol) - (k0 + krow)
            valid = jnp.logical_and(dist >= 0, dist < WIN)
            s = jnp.where(valid, s, -1e30)
            m = jnp.max(s, axis=0, keepdims=True)
            p = jnp.where(valid, jnp.exp2(s - m), 0.0).astype(bf16)
            accs = []
            for j in range(4):
                row0 = pl.multiple_of((g * 4 + j) * HP, HP)
                accs.append(_dot(vtb[pl.ds(row0, HP), pl.ds(k0, 384)], p[:, j * 128:(j + 1) * 128]))
            finish(accs, g, pl.multiple_of(b * 128, 128), None)
            return carry

        lax.fori_loop(0, 64, body, 0)

    def mid(wo_t, proj, src, dst):
        def body(it, carry):
            x_next = out_proj(wo_t, it * UT, src)
            for u in range(UT):
                c = it * UT + u
                tok = pl.ds(pl.multiple_of(c * TC, TC), TC)
                x = x_next
                if u + 1 < UT:
                    x_next = out_proj(wo_t, c + 1, src)
                dst[:, tok] = x
                proj(x, it, u)
            return carry

        lax.fori_loop(0, 2, body, 0)

    def last_body(it, carry):
        xs = [out_proj(wobt, it * UT + u, xb) for u in range(UT)]
        for u in range(UT):
            for k in range(TC // OC):
                c = (it * UT + u) * (TC // OC) + k
                o_stage[:, pl.ds(pl.multiple_of(c * OC, OC), OC)] = xs[u][:, k * OC:(k + 1) * OC].astype(bf16)
                out_copy(c).start()
        return carry

    def network(att):
        fast = att == 0

        def first_body(it, carry):
            @pl.when(jnp.logical_and(fast, it == 1))
            def _():
                x_copy(2).wait()
                x_copy(3).wait()

            nu = 1024 // TF
            for u in range(nu):
                tok = pl.ds(pl.multiple_of((it * nu + u) * TF, TF), TF)
                x = x_in[:, tok].astype(f32)
                xa[:, tok] = x
                proj_a(x, it, u, TF)
            return carry

        lax.fori_loop(0, 2, first_body, 0)

        @pl.when(fast)
        def _():
            cp_wqkv.start()
            cp_wo.wait()
            cp_wob.wait()
            wobt[...] = pltpu.bitcast(wob[...].T, u32)

        def layer_pair(l, carry):
            lax.cond(fast, attn_a_fast, attn_a_safe)

            @pl.when(jnp.logical_and(fast, l == 0))
            def _():
                cp_wqkv.wait()

            mid(woat, proj_b, xa, xb)
            lax.cond(fast, attn_b_fast, attn_b_safe)

            @pl.when(l == 0)
            def _():
                mid(wobt, proj_a, xb, xa)

            return carry

        lax.fori_loop(0, 2, layer_pair, 0)
        lax.fori_loop(0, 2, last_body, 0)
        row = lax.broadcasted_iota(jnp.int32, (8, 128), 0)
        l_ok = jnp.logical_and(lmin_ref[...] > L_LO, lmax_ref[...] < L_HI)
        ok = jnp.logical_and(jnp.logical_or(l_ok, row != DH - 24), vmax_ref[...] < V_HI)
        unsafe = jnp.max(jnp.where(ok, 0.0, 1.0)) > 0.0
        flag[0] = unsafe.astype(jnp.int32)
        for c in range(S // OC):
            out_copy(c).wait()

    def attempt(att, carry):
        @pl.when(flag[0] == 1)
        def _():
            network(att)

        return carry

    lax.fori_loop(0, 2, attempt, 0)


@jax.jit
def pallas_interleave_layers__grouped_kv_mqa__sliding_block__prompt_kernel(
        A_x, A_wq, A_wk, A_wv, A_wo, B_x, B_wqkv, B_wo):
    hbm_spec = pl.BlockSpec(memory_space=pltpu.HBM)
    out_t = pl.pallas_call(
        _kernel,
        out_shape=jax.ShapeDtypeStruct((D, S), bf16),
        in_specs=[hbm_spec] * 7,
        out_specs=hbm_spec,
        scratch_shapes=[
            pltpu.VMEM((D, S), bf16),
            pltpu.VMEM((D, D), bf16),
            pltpu.VMEM((DH, D), bf16),
            pltpu.VMEM((DH, D), bf16),
            pltpu.VMEM((D, D), bf16),
            pltpu.VMEM((D, 3 * D), bf16),
            pltpu.VMEM((D, D), bf16),
            pltpu.VMEM((HP + D // 2, D), u32),
            pltpu.VMEM((D // 2, D), u32),
            pltpu.VMEM((D // 2, D), u32),
            pltpu.VMEM((D, S), f32),
            pltpu.VMEM((D, S), f32),
            pltpu.VMEM((D, S), bf16),
            pltpu.VMEM((4, HP, 4 * S), bf16),
            pltpu.VMEM((4, S // QW, GR, QW), f32),
            pltpu.VMEM((4, 128, 4 * S), bf16),
            pltpu.VMEM((S, 128), bf16),
            pltpu.VMEM((DH, 2 * NV, 128), f32),
            pltpu.VMEM((4, S, 128), bf16),
            pltpu.VMEM((HP, S), bf16),
            pltpu.VMEM((DP, S), bf16),
            pltpu.VMEM((D, S), bf16),
            pltpu.VMEM((16, 256, 128), bf16),
            pltpu.VMEM((HP, S), f32),
            pltpu.VMEM((8, 128), f32),
            pltpu.VMEM((8, 128), f32),
            pltpu.VMEM((8, 128), f32),
            pltpu.SMEM((1,), jnp.int32),
            pltpu.SemaphoreType.DMA((10 + S // OC,)),
        ],
        compiler_params=pltpu.CompilerParams(vmem_limit_bytes=100 * 1024 * 1024),
        name="fused_layers",
    )(A_x.reshape(S, D).T, A_wq, A_wk.T, A_wv.T, A_wo, B_wqkv, B_wo)
    return out_t.T.reshape(1, S, D)
```

```python
import jax
import jax.numpy as jnp
from jax import lax
import jax.experimental.pallas as pl
import jax.experimental.pallas.tpu as pltpu

S = 2048
D = 448
H = 16
DH = 28
HP = 32
DP = H * HP
GR = 4 * DH
WIN = 256
TC = 512
TF = 256
UT = 1024 // TC
NB = TC // 128
UB = 2
OC = 128
QW = 256
EPS = 1e-5
LOG2E = 1.4426950408889634
QSCALE = (DH ** -0.5) * LOG2E
L_LO = 2.0 ** -40
L_HI = 2.0 ** 60
V_HI = 2.0 ** 60
STAGED = (0, 8)
NVS = (96, 80)
NV = max(NVS)
LEAD = 2
DIRECT = [t for t in range(16) if t not in STAGED]
NEG = -1e30

bf16 = jnp.bfloat16
f32 = jnp.float32
u32 = jnp.uint32


def _dot(a, b):
    return jnp.dot(a, b, preferred_element_type=f32)


def _dot_tn(a, b):
    return lax.dot_general(a, b, (((0,), (0,)), ((), ())), preferred_element_type=f32)


def _kernel(x_hbm, wq_hbm, wk_hbm, wv_hbm, wo_hbm, wqkv_hbm, wob_hbm, out_hbm,
            x_in, wq, wk_raw, wv_raw, woa, wqkv, wob,
            wat, woat, wobt, xa, xb, o_stage, qd, qf, qx, ka, kbc, kb, vta, vtb, ot, pbuf, accbuf,
            lmin_ref, lmax_ref, vmax_ref, flag, sems):
    cp_wq = pltpu.make_async_copy(wq_hbm, wq, sems.at[0])
    cp_wk = pltpu.make_async_copy(wk_hbm, wk_raw, sems.at[1])
    cp_wv = pltpu.make_async_copy(wv_hbm, wv_raw, sems.at[2])
    cp_wo = pltpu.make_async_copy(wo_hbm, woa, sems.at[3])
    cp_wqkv = pltpu.make_async_copy(wqkv_hbm, wqkv, sems.at[4])
    cp_wob = pltpu.make_async_copy(wob_hbm, wob, sems.at[5])

    def x_copy(c):
        return pltpu.make_async_copy(x_hbm.at[:, pl.ds(c * 512, 512)], x_in.at[:, pl.ds(c * 512, 512)],
                                     sems.at[6 + c])

    def out_copy(c):
        return pltpu.make_async_copy(o_stage.at[:, pl.ds(c * OC, OC)], out_hbm.at[:, pl.ds(c * OC, OC)],
                                     sems.at[10 + c])

    x_copy(0).start()
    cp_wk.start()
    cp_wv.start()
    cp_wq.start()
    x_copy(1).start()

    pbuf[...] = jnp.zeros(pbuf.shape, bf16)
    accbuf[...] = jnp.ones(accbuf.shape, f32)
    vmax_ref[...] = jnp.zeros(vmax_ref.shape, f32)
    lmin_ref[...] = jnp.ones(lmin_ref.shape, f32)
    lmax_ref[...] = jnp.ones(lmax_ref.shape, f32)

    cp_wk.wait()
    cp_wv.wait()
    zpad = jnp.zeros((HP - DH, D), f32)
    wat[0:HP, :] = pltpu.bitcast(
        jnp.concatenate([wk_raw[...].astype(f32), zpad, wv_raw[...].astype(f32), zpad], axis=0).astype(bf16), u32)
    cp_wq.wait()
    wat[HP:HP + D // 2, :] = pltpu.bitcast(wq[...].T, u32)
    x_copy(0).wait()
    x_copy(1).wait()
    x_copy(2).start()
    x_copy(3).start()
    cp_wo.start()
    cp_wob.start()
    flag[0] = 1

    def layernorm(x):
        outs = []
        for t in range(x.shape[1] // 128):
            xs = x[:, t * 128:(t + 1) * 128]
            m = jnp.mean(xs, axis=0, keepdims=True)
            xc = xs - m
            v = jnp.mean(xc * xc, axis=0, keepdims=True)
            outs.append(xc * lax.rsqrt(v + EPS))
        return jnp.concatenate(outs, axis=1).astype(bf16)

    def v_slab(v):
        row = lax.broadcasted_iota(jnp.int32, v.shape, 0)
        return jnp.where(row < DH, v, jnp.where(row == DH, 1.0, 0.0)).astype(bf16)

    def track_v(v):
        m = vmax_ref[...]
        a = jnp.abs(v)
        for r in range(0, v.shape[0], 8):
            for c0 in range(0, v.shape[1], 128):
                m = jnp.maximum(m, a[r:r + 8, c0:c0 + 128])
        vmax_ref[...] = m

    def proj_a(x, it, u, tc=TC):
        c = it * (1024 // tc) + u
        nb = tc // 128
        tok = pl.ds(pl.multiple_of(c * tc, tc), tc)
        kvq = _dot(pltpu.bitcast(wat[...], bf16), layernorm(x))
        q = kvq[2 * HP:] * QSCALE
        kt = kvq[0:HP]
        kn = jnp.concatenate([kt, kt, kt, kt], axis=0).T
        ka[tok, :] = kn.astype(bf16)
        if u == 0:
            rows = pl.ds(pl.multiple_of(it * NV, 8), NV)
            for d in range(DH):
                kbc[d, rows, :] = jnp.broadcast_to(kn[0:NV, d:d + 1], (NV, 128))
        vta[:, tok] = v_slab(kvq[HP:2 * HP])
        track_v(kvq[HP:2 * HP])
        for k in range(tc // QW):
            for g in range(4):
                qf[g, c * (tc // QW) + k] = q[g * GR:(g + 1) * GR, k * QW:(k + 1) * QW]
        q = jnp.concatenate([q, q[0:8]], axis=0)
        for bb in range(nb):
            for g in range(4):
                col = pl.ds(pl.multiple_of((c * nb + bb) * 512, 512), 512)
                qd[g, :, col] = jnp.concatenate(
                    [q[(g * 4 + j) * DH:(g * 4 + j) * DH + HP, bb * 128:(bb + 1) * 128] for j in range(4)],
                    axis=1).astype(bf16)

    def proj_b(x, it, u):
        c = it * UT + u
        tok = pl.ds(pl.multiple_of(c * TC, TC), TC)
        xn = layernorm(x)
        kt = _dot_tn(wqkv[:, D:2 * D], xn)
        kt = jnp.concatenate([kt, kt[0:16]], axis=0)
        for g in range(4):
            kb[g, tok, :] = kt[g * GR:g * GR + 128, :].T.astype(bf16)
        q = _dot_tn(wqkv[:, 0:D], xn) * QSCALE
        lane_grp = lax.broadcasted_iota(jnp.int32, (8, 128), 1) // 32
        row8 = lax.broadcasted_iota(jnp.int32, (8, 128), 0)
        for bb in range(NB):
            for g in range(4):
                ys = []
                for r in range(0, GR, 8):
                    x8 = q[g * GR + r:g * GR + r + 8, bb * 128:(bb + 1) * 128]
                    j0, j1 = r // DH, (r + 7) // DH
                    y = x8 if j0 == 0 else pltpu.roll(x8, 32 * j0, 1)
                    if j1 != j0:
                        y = jnp.where(row8 < j1 * DH - r, y, pltpu.roll(x8, 32 * j1, 1))
                    ys.append(y)
                qp = pltpu.bitcast(jnp.concatenate(ys, axis=0).astype(bf16), u32)
                tiles = [[] for _ in range(4)]
                for r in range(0, GR // 2, 8):
                    j0, j1 = r // 14, (r + 7) // 14
                    for sb in range(4):
                        keep = lane_grp == (j0 + sb) % 4
                        if j1 != j0:
                            keep = lane_grp == jnp.where(row8 < j1 * 14 - r, (j0 + sb) % 4, (j1 + sb) % 4)
                        tiles[sb].append(jnp.where(keep, qp[r:r + 8], jnp.uint32(0)))
                col = pl.ds(pl.multiple_of((c * NB + bb) * 512, 512), 512)
                qx[g, :, col] = jnp.concatenate([jnp.concatenate(t_, axis=0) for t_ in tiles], axis=1)
        v = _dot_tn(wqkv[:, 2 * D:3 * D], xn)
        track_v(v)
        v = jnp.concatenate([v, v[0:8]], axis=0)
        for h in range(H):
            vtb[h * HP:(h + 1) * HP, tok] = v_slab(v[h * DH:h * DH + HP, :])

    def out_proj(wo_t, c, src):
        tok = pl.ds(pl.multiple_of(c * TC, TC), TC)
        return src[:, tok] + _dot(pltpu.bitcast(wo_t[...], bf16), ot[:, tok])

    def q_tiles(q_ref, g, b, n):
        start = b * 512 if isinstance(b, int) else pl.multiple_of(b * 512, 512)
        return q_ref[g, :, pl.ds(start, 512 * n)]

    def finish(accs, g, col0, stat):
        outs = []
        for acc in accs:
            l = acc[DH:DH + 1, :]
            r = pl.reciprocal(l, approx=True)
            r = r * (2.0 - l * r)
            outs.append(acc[0:DH, :] * r)
            if stat is not None:
                stat = (jnp.minimum(stat[0], acc[24:32, :]), jnp.maximum(stat[1], acc[24:32, :]))
        ot[pl.ds(pl.multiple_of(g * GR, 16), GR), pl.ds(col0, 128)] = jnp.concatenate(outs, axis=0).astype(bf16)
        return stat

    def tiles_k(ts):
        return jnp.concatenate([ka[t * 128:(t + 1) * 128, 0:HP] for t in ts], axis=0)

    def tiles_v(ts):
        return jnp.concatenate([vta[:, t * 128:(t + 1) * 128] for t in ts], axis=1)

    def attn_a_fast():
        def staged_pv(n):
            return accbuf[:, n * 128:(n + 1) * 128] + _dot(tiles_v(STAGED), pbuf[n])

        def body(i, carry):
            g = i // 4
            c = i % 4
            ip = jnp.maximum(i - 1, 0)
            gp = ip // 4
            cp = ip % 4
            stat0 = (lmin_ref[...], lmax_ref[...])
            never = stat0[0] > stat0[1]
            state = {'link': None, 'stat': stat0, 'done': []}

            def finish_prev(n):
                state['done'].append(staged_pv(n))
                if len(state['done']) == 4:
                    col0 = pl.multiple_of((cp * 4 + n // 4) * 128, 128)
                    state['stat'] = finish(state['done'], gp, col0, state['stat'])
                    state['done'] = []

            def vpu_job(n, k, r):
                bb, j = n // 4, n % 4
                k0 = k * NV + r * 16
                qblk = c * (512 // QW) + (bb * 128) // QW
                qcols = pl.ds((bb * 128) % QW, 128)
                a = None
                for d in range(DH):
                    t = kbc[d, k0:k0 + 16, :] * qf[g, qblk, j * DH + d:j * DH + d + 1, qcols]
                    if a is not None:
                        a = a + t
                    elif state['link'] is None:
                        a = t
                    else:
                        lk = state['link']
                        a = jnp.concatenate(
                            [jnp.where(never, lk[8:16], t[0:8]), jnp.where(never, lk[0:8], t[8:16])], axis=0)
                state['link'] = a
                row = k * 128 + r * 16
                pbuf[n, row:row + 16, :] = jnp.exp2(a).astype(bf16)

            jobs = [(n, k, r) for n in range(16) for k in range(2) for r in range(NVS[k] // 16)]
            chunks = [DIRECT[k:k + 2] for k in range(0, len(DIRECT), 2)]
            steps = [(qb, ch) for qb in range(4) for ch in chunks]
            accs = {}
            pend = []

            def pv(qb, ch, s):
                r = _dot(tiles_v(ch), jnp.exp2(s).astype(bf16))
                accs[qb] = r if qb not in accs else accs[qb] + r

            ji = 0
            po = 0
            for t, (qb, ch) in enumerate(steps):
                target = ((t + 1) * len(jobs)) // len(steps)
                need = min(16, jobs[target - 1][0] + 1 + LEAD)
                while po < need:
                    finish_prev(po)
                    po += 1
                pend.append((qb, ch, _dot(tiles_k(ch), q_tiles(qd, g, c * 4 + qb, 1))))
                while ji < target:
                    vpu_job(*jobs[ji])
                    ji += 1
                if t == len(steps) - 1:
                    krest = jnp.concatenate(
                        [ka[st * 128 + NVS[k]:(st + 1) * 128, 0:HP] for k, st in enumerate(STAGED)], axis=0)
                    p = jnp.exp2(_dot(krest, q_tiles(qd, g, c * 4, 4)))
                    for n in range(16):
                        for k in range(2):
                            r0 = k * (128 - NVS[0])
                            pbuf[n, k * 128 + NVS[k]:(k + 1) * 128, :] = (
                                p[r0:r0 + 128 - NVS[k], n * 128:(n + 1) * 128].astype(bf16))
                if len(pend) > 1:
                    pv(*pend.pop(0))
            while pend:
                pv(*pend.pop(0))
            for qb in range(4):
                accbuf[:, qb * 512:(qb + 1) * 512] = accs[qb]
            lmin_ref[...] = jnp.where(i > 0, state['stat'][0], stat0[0])
            lmax_ref[...] = jnp.where(i > 0, state['stat'][1], stat0[1])
            return carry

        lax.fori_loop(0, 16, body, 0)
        woat[...] = pltpu.bitcast(woa[...].T, u32)
        stat = (lmin_ref[...], lmax_ref[...])
        for bb in range(4):
            stat = finish([staged_pv(bb * 4 + j) for j in range(4)], 3, (12 + bb) * 128, stat)
        lmin_ref[...] = stat[0]
        lmax_ref[...] = stat[1]

    def attn_a_safe():
        def body(i, carry):
            g = i // 16
            b = i % 16
            s = _dot(ka[:, 0:HP], q_tiles(qd, g, b, 1))
            m = jnp.max(s, axis=0, keepdims=True)
            p = jnp.exp2(s - m).astype(bf16)
            acc = _dot(vta[...], p)
            finish([acc[:, j * 128:(j + 1) * 128] for j in range(4)], g, pl.multiple_of(b * 128, 128), None)
            return carry

        lax.fori_loop(0, 64, body, 0)

    def unrotate(acc, j):
        return acc if j == 0 else pltpu.roll(acc, 128 - 32 * j, 1)

    def attn_b_fast():
        lane = lax.broadcasted_iota(jnp.int32, (32, 128), 1)
        diag = lax.broadcasted_iota(jnp.int32, (32, 128), 0) <= (lane & 31)
        odd = (lane & 32) != 0
        high = lane >= 64
        fill = jnp.full((32, 128), NEG, f32)

        def sel(m, a_, b_):
            if a_ is None and b_ is None:
                return None
            return jnp.where(m, fill if a_ is None else a_, fill if b_ is None else b_)

        def body(it, carry):
            stat = (lmin_ref[...], lmax_ref[...])

            def qk(g, b):
                outs = []
                for sb in range(4):
                    hi = b * 128 + sb * 32 + 32
                    lo = max(hi - 288, 0)
                    w = pltpu.bitcast(qx[g, :, (b * 4 + sb) * 128:(b * 4 + sb + 1) * 128], bf16)
                    outs.append(_dot(kb[g, lo:hi, 0:GR], w))
                return outs

            items = [(it * UB + u, b) for u in range(UB) for b in range(16)]
            s_next = qk(*items[0])
            for n, (g, b) in enumerate(items):
                ss = s_next
                if n + 1 < len(items):
                    s_next = qk(*items[n + 1])
                e = []
                for sb in range(4):
                    top = b * 4 + sb
                    first = max(top - 8, 0)
                    d = {first + t: ss[sb][t * 32:(t + 1) * 32] for t in range(top - first + 1)}
                    d[top] = jnp.where(diag, d[top], NEG)
                    if top - 8 >= 0:
                        d[top - 8] = jnp.where(diag, NEG, d[top - 8])
                    e.append(d)
                lo_t = max(b - 2, 0)
                pj = [[] for _ in range(4)]
                for rho in range(lo_t * 4, (b + 1) * 4):
                    src = [e[sb].get(rho) for sb in range(4)]
                    t1 = [sel(odd, src[(sb + 1) % 4], src[sb]) for sb in range(4)]
                    for j in range(4):
                        s0 = (-j) % 4
                        pj[j].append(jnp.exp2(sel(high, t1[(s0 + 2) % 4], t1[s0])))
                accs = [None] * 4
                for t in range(lo_t, b + 1):
                    for j in range(4):
                        row0 = pl.multiple_of((g * 4 + j) * HP, HP)
                        p = jnp.concatenate(pj[j][(t - lo_t) * 4:(t - lo_t + 1) * 4], axis=0).astype(bf16)
                        pv = _dot(vtb[pl.ds(row0, HP), t * 128:(t + 1) * 128], p)
                        accs[j] = pv if accs[j] is None else accs[j] + pv
                stat = finish([unrotate(acc, j) for j, acc in enumerate(accs)], g, b * 128, stat)
            lmin_ref[...] = stat[0]
            lmax_ref[...] = stat[1]
            return carry

        lax.fori_loop(0, 4 // UB, body, 0)

    def attn_b_safe():
        krow = lax.broadcasted_iota(jnp.int32, (384, 512), 0)
        col = lax.broadcasted_iota(jnp.int32, (384, 512), 1)
        qoff = (col // 128) * 32 + (col & 31)
        lane_grp = lax.broadcasted_iota(jnp.int32, (HP, 128), 1) // 32

        def body(i, carry):
            g = i // 16
            b = i % 16
            k0 = pl.multiple_of(jnp.maximum(b - 2, 0) * 128, 128)
            s = _dot(kb[g, pl.ds(k0, 384), 0:GR], pltpu.bitcast(q_tiles(qx, g, b, 1), bf16))
            dist = (b * 128 + qoff) - (k0 + krow)
            valid = jnp.logical_and(dist >= 0, dist < WIN)
            s = jnp.where(valid, s, NEG)
            m = jnp.max(s, axis=0, keepdims=True)
            p = jnp.where(valid, jnp.exp2(s - m), 0.0).astype(bf16)
            o = _dot(vtb[pl.ds(pl.multiple_of(g * 128, 128), 128), pl.ds(k0, 384)], p)
            accs = []
            for j in range(4):
                acc = o[j * HP:(j + 1) * HP, 0:128]
                for sb in range(1, 4):
                    acc = jnp.where(lane_grp == (j + sb) % 4, o[j * HP:(j + 1) * HP, sb * 128:(sb + 1) * 128], acc)
                accs.append(unrotate(acc, j))
            finish(accs, g, pl.multiple_of(b * 128, 128), None)
            return carry

        lax.fori_loop(0, 64, body, 0)

    def mid(wo_t, proj, src, dst):
        def body(it, carry):
            x_next = out_proj(wo_t, it * UT, src)
            for u in range(UT):
                c = it * UT + u
                tok = pl.ds(pl.multiple_of(c * TC, TC), TC)
                x = x_next
                if u + 1 < UT:
                    x_next = out_proj(wo_t, c + 1, src)
                dst[:, tok] = x
                proj(x, it, u)
            return carry

        lax.fori_loop(0, 2, body, 0)

    def last_body(it, carry):
        xs = [out_proj(wobt, it * UT + u, xb) for u in range(UT)]
        for u in range(UT):
            for k in range(TC // OC):
                c = (it * UT + u) * (TC // OC) + k
                o_stage[:, pl.ds(pl.multiple_of(c * OC, OC), OC)] = xs[u][:, k * OC:(k + 1) * OC].astype(bf16)
                out_copy(c).start()
        return carry

    def network(att):
        fast = att == 0

        def first_body(it, carry):
            @pl.when(jnp.logical_and(fast, it == 1))
            def _():
                x_copy(2).wait()
                x_copy(3).wait()

            nu = 1024 // TF
            for u in range(nu):
                tok = pl.ds(pl.multiple_of((it * nu + u) * TF, TF), TF)
                x = x_in[:, tok].astype(f32)
                xa[:, tok] = x
                proj_a(x, it, u, TF)
            return carry

        lax.fori_loop(0, 2, first_body, 0)

        @pl.when(fast)
        def _():
            cp_wqkv.start()
            cp_wo.wait()
            cp_wob.wait()
            wobt[...] = pltpu.bitcast(wob[...].T, u32)

        def layer_pair(l, carry):
            lax.cond(fast, attn_a_fast, attn_a_safe)

            @pl.when(jnp.logical_and(fast, l == 0))
            def _():
                cp_wqkv.wait()

            mid(woat, proj_b, xa, xb)
            lax.cond(fast, attn_b_fast, attn_b_safe)

            @pl.when(l == 0)
            def _():
                mid(wobt, proj_a, xb, xa)

            return carry

        lax.fori_loop(0, 2, layer_pair, 0)
        lax.fori_loop(0, 2, last_body, 0)
        row = lax.broadcasted_iota(jnp.int32, (8, 128), 0)
        l_ok = jnp.logical_and(lmin_ref[...] > L_LO, lmax_ref[...] < L_HI)
        ok = jnp.logical_and(jnp.logical_or(l_ok, row != DH - 24), vmax_ref[...] < V_HI)
        unsafe = jnp.max(jnp.where(ok, 0.0, 1.0)) > 0.0
        flag[0] = unsafe.astype(jnp.int32)
        for c in range(S // OC):
            out_copy(c).wait()

    def attempt(att, carry):
        @pl.when(flag[0] == 1)
        def _():
            network(att)

        return carry

    lax.fori_loop(0, 2, attempt, 0)


@jax.jit
def pallas_interleave_layers__grouped_kv_mqa__sliding_block__prompt_kernel(
        A_x, A_wq, A_wk, A_wv, A_wo, B_x, B_wqkv, B_wo):
    hbm_spec = pl.BlockSpec(memory_space=pltpu.HBM)
    out_t = pl.pallas_call(
        _kernel,
        out_shape=jax.ShapeDtypeStruct((D, S), bf16),
        in_specs=[hbm_spec] * 7,
        out_specs=hbm_spec,
        scratch_shapes=[
            pltpu.VMEM((D, S), bf16),
            pltpu.VMEM((D, D), bf16),
            pltpu.VMEM((DH, D), bf16),
            pltpu.VMEM((DH, D), bf16),
            pltpu.VMEM((D, D), bf16),
            pltpu.VMEM((D, 3 * D), bf16),
            pltpu.VMEM((D, D), bf16),
            pltpu.VMEM((HP + D // 2, D), u32),
            pltpu.VMEM((D // 2, D), u32),
            pltpu.VMEM((D // 2, D), u32),
            pltpu.VMEM((D, S), f32),
            pltpu.VMEM((D, S), f32),
            pltpu.VMEM((D, S), bf16),
            pltpu.VMEM((4, HP, 4 * S), bf16),
            pltpu.VMEM((4, S // QW, GR, QW), f32),
            pltpu.VMEM((4, GR // 2, 4 * S), u32),
            pltpu.VMEM((S, 128), bf16),
            pltpu.VMEM((DH, 2 * NV, 128), f32),
            pltpu.VMEM((4, S, 128), bf16),
            pltpu.VMEM((HP, S), bf16),
            pltpu.VMEM((DP, S), bf16),
            pltpu.VMEM((D, S), bf16),
            pltpu.VMEM((16, 256, 128), bf16),
            pltpu.VMEM((HP, S), f32),
            pltpu.VMEM((8, 128), f32),
            pltpu.VMEM((8, 128), f32),
            pltpu.VMEM((8, 128), f32),
            pltpu.SMEM((1,), jnp.int32),
            pltpu.SemaphoreType.DMA((10 + S // OC,)),
        ],
        compiler_params=pltpu.CompilerParams(vmem_limit_bytes=100 * 1024 * 1024),
        name="fused_layers",
    )(A_x.reshape(S, D).T, A_wq, A_wk.T, A_wv.T, A_wo, B_wqkv, B_wo)
    return out_t.T.reshape(1, S, D)
```

```python
import jax
import jax.numpy as jnp
from jax import lax
import jax.experimental.pallas as pl
import jax.experimental.pallas.tpu as pltpu

S = 2048
D = 448
H = 16
DH = 28
HP = 32
DP = H * HP
GR = 4 * DH
WIN = 256
TC = 512
TF = 256
UT = 1024 // TC
NB = TC // 128
UB = 2
OC = 128
QW = 256
EPS = 1e-5
LOG2E = 1.4426950408889634
QSCALE = (DH ** -0.5) * LOG2E
L_LO = 2.0 ** -40
L_HI = 2.0 ** 60
V_HI = 2.0 ** 60
STAGED = (0, 8)
NVS = (96, 80)
NV = max(NVS)
LEAD = 2
DIRECT = [t for t in range(16) if t not in STAGED]
NEG = -1e30

bf16 = jnp.bfloat16
f32 = jnp.float32
u32 = jnp.uint32


def _dot(a, b):
    return jnp.dot(a, b, preferred_element_type=f32)


def _dot_tn(a, b):
    return lax.dot_general(a, b, (((0,), (0,)), ((), ())), preferred_element_type=f32)


def _kernel(x_hbm, wq_hbm, wk_hbm, wv_hbm, wo_hbm, wqkv_hbm, wob_hbm, out_hbm,
            x_in, wq, wk_raw, wv_raw, woa, wqkv, wob,
            wat, woat, wobt, xa, xb, o_stage, qd, qf, qx, ka, kbc, kb, vta, vtb, ot, pbuf, accbuf,
            lmin_ref, lmax_ref, vmax_ref, flag, sems):
    cp_wq = pltpu.make_async_copy(wq_hbm, wq, sems.at[0])
    cp_wk = pltpu.make_async_copy(wk_hbm, wk_raw, sems.at[1])
    cp_wv = pltpu.make_async_copy(wv_hbm, wv_raw, sems.at[2])
    cp_wo = pltpu.make_async_copy(wo_hbm, woa, sems.at[3])
    cp_wqkv = pltpu.make_async_copy(wqkv_hbm, wqkv, sems.at[4])
    cp_wob = pltpu.make_async_copy(wob_hbm, wob, sems.at[5])

    def x_copy(c):
        return pltpu.make_async_copy(x_hbm.at[:, pl.ds(c * 512, 512)], x_in.at[:, pl.ds(c * 512, 512)],
                                     sems.at[6 + c])

    def out_copy(c):
        return pltpu.make_async_copy(o_stage.at[:, pl.ds(c * OC, OC)], out_hbm.at[:, pl.ds(c * OC, OC)],
                                     sems.at[10])

    x_copy(0).start()
    cp_wk.start()
    cp_wv.start()
    cp_wq.start()
    x_copy(1).start()

    pbuf[...] = jnp.zeros(pbuf.shape, bf16)
    accbuf[...] = jnp.ones(accbuf.shape, f32)
    vmax_ref[...] = jnp.zeros(vmax_ref.shape, f32)
    lmin_ref[...] = jnp.ones(lmin_ref.shape, f32)
    lmax_ref[...] = jnp.ones(lmax_ref.shape, f32)

    cp_wk.wait()
    cp_wv.wait()
    zpad = jnp.zeros((HP - DH, D), f32)
    wat[0:HP, :] = pltpu.bitcast(
        jnp.concatenate([wk_raw[...].astype(f32), zpad, wv_raw[...].astype(f32), zpad], axis=0).astype(bf16), u32)
    cp_wq.wait()
    wat[HP:HP + D // 2, :] = pltpu.bitcast(wq[...].T, u32)
    x_copy(0).wait()
    x_copy(1).wait()
    x_copy(2).start()
    x_copy(3).start()
    cp_wo.start()
    cp_wob.start()
    flag[0] = 1

    def layernorm(x):
        outs = []
        for t in range(x.shape[1] // 128):
            xs = x[:, t * 128:(t + 1) * 128]
            m = jnp.mean(xs, axis=0, keepdims=True)
            xc = xs - m
            v = jnp.mean(xc * xc, axis=0, keepdims=True)
            outs.append(xc * lax.rsqrt(v + EPS))
        return jnp.concatenate(outs, axis=1).astype(bf16)

    def v_slab(v):
        row = lax.broadcasted_iota(jnp.int32, v.shape, 0)
        return jnp.where(row < DH, v, jnp.where(row == DH, 1.0, 0.0)).astype(bf16)

    def track_v(v):
        m = vmax_ref[...]
        a = jnp.abs(v)
        for r in range(0, v.shape[0], 8):
            for c0 in range(0, v.shape[1], 128):
                m = jnp.maximum(m, a[r:r + 8, c0:c0 + 128])
        vmax_ref[...] = m

    def proj_a(x, it, u, tc=TC):
        c = it * (1024 // tc) + u
        nb = tc // 128
        tok = pl.ds(pl.multiple_of(c * tc, tc), tc)
        kvq = _dot(pltpu.bitcast(wat[...], bf16), layernorm(x))
        q = kvq[2 * HP:] * QSCALE
        kt = kvq[0:HP]
        kn = jnp.concatenate([kt, kt, kt, kt], axis=0).T
        ka[tok, :] = kn.astype(bf16)
        if u == 0:
            rows = pl.ds(pl.multiple_of(it * NV, 8), NV)
            for d in range(DH):
                kbc[d, rows, :] = jnp.broadcast_to(kn[0:NV, d:d + 1], (NV, 128))
        vta[:, tok] = v_slab(kvq[HP:2 * HP])
        track_v(kvq[HP:2 * HP])
        for k in range(tc // QW):
            for g in range(4):
                qf[g, c * (tc // QW) + k] = q[g * GR:(g + 1) * GR, k * QW:(k + 1) * QW]
        q = jnp.concatenate([q, q[0:8]], axis=0)
        for bb in range(nb):
            for g in range(4):
                col = pl.ds(pl.multiple_of((c * nb + bb) * 512, 512), 512)
                qd[g, :, col] = jnp.concatenate(
                    [q[(g * 4 + j) * DH:(g * 4 + j) * DH + HP, bb * 128:(bb + 1) * 128] for j in range(4)],
                    axis=1).astype(bf16)

    def proj_b(x, it, u):
        c = it * UT + u
        tok = pl.ds(pl.multiple_of(c * TC, TC), TC)
        xn = layernorm(x)
        kt = _dot_tn(wqkv[:, D:2 * D], xn)
        kt = jnp.concatenate([kt, kt[0:16]], axis=0)
        for g in range(4):
            kb[g, tok, :] = kt[g * GR:g * GR + 128, :].T.astype(bf16)
        q = _dot_tn(wqkv[:, 0:D], xn) * QSCALE
        lane_grp = lax.broadcasted_iota(jnp.int32, (8, 128), 1) // 32
        row8 = lax.broadcasted_iota(jnp.int32, (8, 128), 0)
        for bb in range(NB):
            for g in range(4):
                ys = []
                for r in range(0, GR, 8):
                    x8 = q[g * GR + r:g * GR + r + 8, bb * 128:(bb + 1) * 128]
                    j0, j1 = r // DH, (r + 7) // DH
                    y = x8 if j0 == 0 else pltpu.roll(x8, 32 * j0, 1)
                    if j1 != j0:
                        y = jnp.where(row8 < j1 * DH - r, y, pltpu.roll(x8, 32 * j1, 1))
                    ys.append(y)
                qp = pltpu.bitcast(jnp.concatenate(ys, axis=0).astype(bf16), u32)
                tiles = [[] for _ in range(4)]
                for r in range(0, GR // 2, 8):
                    j0, j1 = r // 14, (r + 7) // 14
                    for sb in range(4):
                        keep = lane_grp == (j0 + sb) % 4
                        if j1 != j0:
                            keep = lane_grp == jnp.where(row8 < j1 * 14 - r, (j0 + sb) % 4, (j1 + sb) % 4)
                        tiles[sb].append(jnp.where(keep, qp[r:r + 8], jnp.uint32(0)))
                col = pl.ds(pl.multiple_of((c * NB + bb) * 512, 512), 512)
                qx[g, :, col] = jnp.concatenate([jnp.concatenate(t_, axis=0) for t_ in tiles], axis=1)
        v = _dot_tn(wqkv[:, 2 * D:3 * D], xn)
        track_v(v)
        v = jnp.concatenate([v, v[0:8]], axis=0)
        for h in range(H):
            vtb[h * HP:(h + 1) * HP, tok] = v_slab(v[h * DH:h * DH + HP, :])

    def out_proj(wo_t, c, src):
        tok = pl.ds(pl.multiple_of(c * TC, TC), TC)
        return src[:, tok] + _dot(pltpu.bitcast(wo_t[...], bf16), ot[:, tok])

    def q_tiles(q_ref, g, b, n):
        start = b * 512 if isinstance(b, int) else pl.multiple_of(b * 512, 512)
        return q_ref[g, :, pl.ds(start, 512 * n)]

    def finish(accs, g, col0, stat):
        outs = []
        for acc in accs:
            l = acc[DH:DH + 1, :]
            r = pl.reciprocal(l, approx=True)
            r = r * (2.0 - l * r)
            outs.append(acc[0:DH, :] * r)
            if stat is not None:
                stat = (jnp.minimum(stat[0], acc[24:32, :]), jnp.maximum(stat[1], acc[24:32, :]))
        ot[pl.ds(pl.multiple_of(g * GR, 16), GR), pl.ds(col0, 128)] = jnp.concatenate(outs, axis=0).astype(bf16)
        return stat

    def tiles_k(ts):
        return jnp.concatenate([ka[t * 128:(t + 1) * 128, 0:HP] for t in ts], axis=0)

    def tiles_v(ts):
        return jnp.concatenate([vta[:, t * 128:(t + 1) * 128] for t in ts], axis=1)

    def attn_a_fast():
        def staged_pv(n):
            return accbuf[:, n * 128:(n + 1) * 128] + _dot(tiles_v(STAGED), pbuf[n])

        def body(i, carry):
            g = i // 4
            c = i % 4
            ip = jnp.maximum(i - 1, 0)
            gp = ip // 4
            cp = ip % 4
            stat0 = (lmin_ref[...], lmax_ref[...])
            never = stat0[0] > stat0[1]
            state = {'link': None, 'stat': stat0, 'done': []}

            def finish_prev(n):
                state['done'].append(staged_pv(n))
                if len(state['done']) == 4:
                    col0 = pl.multiple_of((cp * 4 + n // 4) * 128, 128)
                    state['stat'] = finish(state['done'], gp, col0, state['stat'])
                    state['done'] = []

            def vpu_job(n, k, r):
                bb, j = n // 4, n % 4
                k0 = k * NV + r * 16
                qblk = c * (512 // QW) + (bb * 128) // QW
                qcols = pl.ds((bb * 128) % QW, 128)
                a = None
                for d in range(DH):
                    t = kbc[d, k0:k0 + 16, :] * qf[g, qblk, j * DH + d:j * DH + d + 1, qcols]
                    if a is not None:
                        a = a + t
                    elif state['link'] is None:
                        a = t
                    else:
                        lk = state['link']
                        a = jnp.concatenate(
                            [jnp.where(never, lk[8:16], t[0:8]), jnp.where(never, lk[0:8], t[8:16])], axis=0)
                state['link'] = a
                row = k * 128 + r * 16
                pbuf[n, row:row + 16, :] = jnp.exp2(a).astype(bf16)

            jobs = [(n, k, r) for n in range(16) for k in range(2) for r in range(NVS[k] // 16)]
            chunks = [DIRECT[k:k + 2] for k in range(0, len(DIRECT), 2)]
            steps = [(qb, ch) for qb in range(4) for ch in chunks]
            accs = {}
            pend = []

            def pv(qb, ch, s):
                r = _dot(tiles_v(ch), jnp.exp2(s).astype(bf16))
                accs[qb] = r if qb not in accs else accs[qb] + r

            ji = 0
            po = 0
            for t, (qb, ch) in enumerate(steps):
                target = ((t + 1) * len(jobs)) // len(steps)
                need = min(16, jobs[target - 1][0] + 1 + LEAD)
                while po < need:
                    finish_prev(po)
                    po += 1
                pend.append((qb, ch, _dot(tiles_k(ch), q_tiles(qd, g, c * 4 + qb, 1))))
                while ji < target:
                    vpu_job(*jobs[ji])
                    ji += 1
                if t == len(steps) - 1:
                    krest = jnp.concatenate(
                        [ka[st * 128 + NVS[k]:(st + 1) * 128, 0:HP] for k, st in enumerate(STAGED)], axis=0)
                    p = jnp.exp2(_dot(krest, q_tiles(qd, g, c * 4, 4)))
                    for n in range(16):
                        for k in range(2):
                            r0 = k * (128 - NVS[0])
                            pbuf[n, k * 128 + NVS[k]:(k + 1) * 128, :] = (
                                p[r0:r0 + 128 - NVS[k], n * 128:(n + 1) * 128].astype(bf16))
                if len(pend) > 1:
                    pv(*pend.pop(0))
            while pend:
                pv(*pend.pop(0))
            for qb in range(4):
                accbuf[:, qb * 512:(qb + 1) * 512] = accs[qb]
            lmin_ref[...] = jnp.where(i > 0, state['stat'][0], stat0[0])
            lmax_ref[...] = jnp.where(i > 0, state['stat'][1], stat0[1])
            return carry

        lax.fori_loop(0, 16, body, 0)
        woat[...] = pltpu.bitcast(woa[...].T, u32)
        stat = (lmin_ref[...], lmax_ref[...])
        for bb in range(4):
            stat = finish([staged_pv(bb * 4 + j) for j in range(4)], 3, (12 + bb) * 128, stat)
        lmin_ref[...] = stat[0]
        lmax_ref[...] = stat[1]

    def attn_a_safe():
        def body(i, carry):
            g = i // 16
            b = i % 16
            s = _dot(ka[:, 0:HP], q_tiles(qd, g, b, 1))
            m = jnp.max(s, axis=0, keepdims=True)
            p = jnp.exp2(s - m).astype(bf16)
            acc = _dot(vta[...], p)
            finish([acc[:, j * 128:(j + 1) * 128] for j in range(4)], g, pl.multiple_of(b * 128, 128), None)
            return carry

        lax.fori_loop(0, 64, body, 0)

    def unrotate(acc, j):
        return acc if j == 0 else pltpu.roll(acc, 128 - 32 * j, 1)

    def attn_b_fast():
        lane = lax.broadcasted_iota(jnp.int32, (32, 128), 1)
        diag = lax.broadcasted_iota(jnp.int32, (32, 128), 0) <= (lane & 31)
        odd = (lane & 32) != 0
        high = lane >= 64
        fill = jnp.full((32, 128), NEG, f32)

        def sel(m, a_, b_):
            if a_ is None and b_ is None:
                return None
            return jnp.where(m, fill if a_ is None else a_, fill if b_ is None else b_)

        def body(it, carry):
            stat = (lmin_ref[...], lmax_ref[...])

            def qk(g, b):
                outs = []
                for sb in range(4):
                    hi = b * 128 + sb * 32 + 32
                    lo = max(hi - 288, 0)
                    w = pltpu.bitcast(qx[g, :, (b * 4 + sb) * 128:(b * 4 + sb + 1) * 128], bf16)
                    outs.append(_dot(kb[g, lo:hi, 0:GR], w))
                return outs

            items = [(it * UB + u, b) for u in range(UB) for b in range(16)]
            s_next = qk(*items[0])
            for n, (g, b) in enumerate(items):
                ss = s_next
                if n + 1 < len(items):
                    s_next = qk(*items[n + 1])
                e = []
                for sb in range(4):
                    top = b * 4 + sb
                    first = max(top - 8, 0)
                    d = {first + t: ss[sb][t * 32:(t + 1) * 32] for t in range(top - first + 1)}
                    d[top] = jnp.where(diag, d[top], NEG)
                    if top - 8 >= 0:
                        d[top - 8] = jnp.where(diag, NEG, d[top - 8])
                    e.append(d)
                lo_t = max(b - 2, 0)
                pj = [[] for _ in range(4)]
                for rho in range(lo_t * 4, (b + 1) * 4):
                    src = [e[sb].get(rho) for sb in range(4)]
                    t1 = [sel(odd, src[(sb + 1) % 4], src[sb]) for sb in range(4)]
                    for j in range(4):
                        s0 = (-j) % 4
                        pj[j].append(jnp.exp2(sel(high, t1[(s0 + 2) % 4], t1[s0])))
                accs = [None] * 4
                for t in range(lo_t, b + 1):
                    for j in range(4):
                        row0 = pl.multiple_of((g * 4 + j) * HP, HP)
                        p = jnp.concatenate(pj[j][(t - lo_t) * 4:(t - lo_t + 1) * 4], axis=0).astype(bf16)
                        pv = _dot(vtb[pl.ds(row0, HP), t * 128:(t + 1) * 128], p)
                        accs[j] = pv if accs[j] is None else accs[j] + pv
                stat = finish([unrotate(acc, j) for j, acc in enumerate(accs)], g, b * 128, stat)
            lmin_ref[...] = stat[0]
            lmax_ref[...] = stat[1]
            return carry

        lax.fori_loop(0, 4 // UB, body, 0)

    def attn_b_safe():
        krow = lax.broadcasted_iota(jnp.int32, (384, 512), 0)
        col = lax.broadcasted_iota(jnp.int32, (384, 512), 1)
        qoff = (col // 128) * 32 + (col & 31)
        lane_grp = lax.broadcasted_iota(jnp.int32, (HP, 128), 1) // 32

        def body(i, carry):
            g = i // 16
            b = i % 16
            k0 = pl.multiple_of(jnp.maximum(b - 2, 0) * 128, 128)
            s = _dot(kb[g, pl.ds(k0, 384), 0:GR], pltpu.bitcast(q_tiles(qx, g, b, 1), bf16))
            dist = (b * 128 + qoff) - (k0 + krow)
            valid = jnp.logical_and(dist >= 0, dist < WIN)
            s = jnp.where(valid, s, NEG)
            m = jnp.max(s, axis=0, keepdims=True)
            p = jnp.where(valid, jnp.exp2(s - m), 0.0).astype(bf16)
            o = _dot(vtb[pl.ds(pl.multiple_of(g * 128, 128), 128), pl.ds(k0, 384)], p)
            accs = []
            for j in range(4):
                acc = o[j * HP:(j + 1) * HP, 0:128]
                for sb in range(1, 4):
                    acc = jnp.where(lane_grp == (j + sb) % 4, o[j * HP:(j + 1) * HP, sb * 128:(sb + 1) * 128], acc)
                accs.append(unrotate(acc, j))
            finish(accs, g, pl.multiple_of(b * 128, 128), None)
            return carry

        lax.fori_loop(0, 64, body, 0)

    def mid(wo_t, proj, src, dst):
        def body(it, carry):
            x_next = out_proj(wo_t, it * UT, src)
            for u in range(UT):
                c = it * UT + u
                tok = pl.ds(pl.multiple_of(c * TC, TC), TC)
                x = x_next
                if u + 1 < UT:
                    x_next = out_proj(wo_t, c + 1, src)
                dst[:, tok] = x
                proj(x, it, u)
            return carry

        lax.fori_loop(0, 2, body, 0)

    def last_body(it, carry):
        xs = [out_proj(wobt, it * UT + u, xb) for u in range(UT)]
        for u in range(UT):
            for k in range(TC // OC):
                c = (it * UT + u) * (TC // OC) + k
                o_stage[:, pl.ds(pl.multiple_of(c * OC, OC), OC)] = xs[u][:, k * OC:(k + 1) * OC].astype(bf16)
                out_copy(c).start()
        return carry

    def network(att):
        fast = att == 0

        def first_body(it, carry):
            @pl.when(jnp.logical_and(fast, it == 1))
            def _():
                x_copy(2).wait()
                x_copy(3).wait()

            nu = 1024 // TF
            for u in range(nu):
                tok = pl.ds(pl.multiple_of((it * nu + u) * TF, TF), TF)
                x = x_in[:, tok].astype(f32)
                xa[:, tok] = x
                proj_a(x, it, u, TF)
            return carry

        lax.fori_loop(0, 2, first_body, 0)

        @pl.when(fast)
        def _():
            cp_wqkv.start()
            cp_wo.wait()
            cp_wob.wait()
            wobt[...] = pltpu.bitcast(wob[...].T, u32)

        def layer_pair(l, carry):
            lax.cond(fast, attn_a_fast, attn_a_safe)

            @pl.when(jnp.logical_and(fast, l == 0))
            def _():
                cp_wqkv.wait()

            mid(woat, proj_b, xa, xb)
            lax.cond(fast, attn_b_fast, attn_b_safe)

            @pl.when(l == 0)
            def _():
                mid(wobt, proj_a, xb, xa)

            return carry

        lax.fori_loop(0, 2, layer_pair, 0)
        lax.fori_loop(0, 2, last_body, 0)
        row = lax.broadcasted_iota(jnp.int32, (8, 128), 0)
        l_ok = jnp.logical_and(lmin_ref[...] > L_LO, lmax_ref[...] < L_HI)
        ok = jnp.logical_and(jnp.logical_or(l_ok, row != DH - 24), vmax_ref[...] < V_HI)
        unsafe = jnp.max(jnp.where(ok, 0.0, 1.0)) > 0.0
        flag[0] = unsafe.astype(jnp.int32)
        pltpu.make_async_copy(o_stage, out_hbm, sems.at[10]).wait()

    def attempt(att, carry):
        @pl.when(flag[0] == 1)
        def _():
            network(att)

        return carry

    lax.fori_loop(0, 2, attempt, 0)


@jax.jit
def pallas_interleave_layers__grouped_kv_mqa__sliding_block__prompt_kernel(
        A_x, A_wq, A_wk, A_wv, A_wo, B_x, B_wqkv, B_wo):
    hbm_spec = pl.BlockSpec(memory_space=pltpu.HBM)
    out_t = pl.pallas_call(
        _kernel,
        out_shape=jax.ShapeDtypeStruct((D, S), bf16),
        in_specs=[hbm_spec] * 7,
        out_specs=hbm_spec,
        scratch_shapes=[
            pltpu.VMEM((D, S), bf16),
            pltpu.VMEM((D, D), bf16),
            pltpu.VMEM((DH, D), bf16),
            pltpu.VMEM((DH, D), bf16),
            pltpu.VMEM((D, D), bf16),
            pltpu.VMEM((D, 3 * D), bf16),
            pltpu.VMEM((D, D), bf16),
            pltpu.VMEM((HP + D // 2, D), u32),
            pltpu.VMEM((D // 2, D), u32),
            pltpu.VMEM((D // 2, D), u32),
            pltpu.VMEM((D, S), f32),
            pltpu.VMEM((D, S), f32),
            pltpu.VMEM((D, S), bf16),
            pltpu.VMEM((4, HP, 4 * S), bf16),
            pltpu.VMEM((4, S // QW, GR, QW), f32),
            pltpu.VMEM((4, GR // 2, 4 * S), u32),
            pltpu.VMEM((S, 128), bf16),
            pltpu.VMEM((DH, 2 * NV, 128), f32),
            pltpu.VMEM((4, S, 128), bf16),
            pltpu.VMEM((HP, S), bf16),
            pltpu.VMEM((DP, S), bf16),
            pltpu.VMEM((D, S), bf16),
            pltpu.VMEM((16, 256, 128), bf16),
            pltpu.VMEM((HP, S), f32),
            pltpu.VMEM((8, 128), f32),
            pltpu.VMEM((8, 128), f32),
            pltpu.VMEM((8, 128), f32),
            pltpu.SMEM((1,), jnp.int32),
            pltpu.SemaphoreType.DMA((11,)),
        ],
        compiler_params=pltpu.CompilerParams(vmem_limit_bytes=100 * 1024 * 1024),
        name="fused_layers",
    )(A_x.reshape(S, D).T, A_wq, A_wk.T, A_wv.T, A_wo, B_wqkv, B_wo)
    return out_t.T.reshape(1, S, D)
```
